```python
import jax
import jax.numpy as jnp

def _softmax(x, axis=-1):
    return jax.nn.softmax(x, axis=axis)
def _gelu(x):
    return jax.nn.gelu(x, approximate=True)
def _silu(x):
    return jax.nn.silu(x)
def _sigmoid(x):
    return jax.nn.sigmoid(x)
def _layernorm(x, axis=-1, eps=1e-5):
    m = jnp.mean(x, axis=axis, keepdims=True)
    v = jnp.var(x, axis=axis, keepdims=True)
    return (x - m) / jnp.sqrt(v + eps)
def _scatter_add(tgt, idx, src, axis=0):
    return tgt.at[idx].add(src)
def _segment_sum(src, seg, n):
    return jax.ops.segment_sum(src, seg, n)
class _Rng:
    def __init__(self, key):
        self._k = key
    def _next(self):
        self._k, sub = jax.random.split(self._k)
        return sub
    def normal(self, shape):
        return jax.random.normal(self._next(), shape, dtype=jnp.bfloat16)
    def randint(self, lo, hi, shape):
        return jax.random.randint(self._next(), shape, lo, hi, dtype=jnp.int32)
    def uniform(self, shape, lo=0.0, hi=1.0):
        return jax.random.uniform(self._next(), shape, jnp.bfloat16, lo, hi)
    def permutation(self, n):
        return jax.random.permutation(self._next(), n)


kernel_name = 'standalone__structured_sparse_n_m__ragged'

def setup_inputs():
    _rng = _Rng(jax.random.key(int.from_bytes(__import__("os").urandom(4), "little")))
    _w = (lambda a: (lambda t: t.astype(jnp.bfloat16) if jnp.issubdtype(t.dtype, jnp.floating) else t)(jnp.asarray(a)))
    B, S, D = 16, 4096, 576
    assert D % 4 == 0, "d_model must be divisible by M=4 for 2:4 sparsity"
    return {
        "x": _w((lambda *s: _rng.normal(s) * 0.05)(B, S, D)),
        "w": _w((lambda *s: _rng.normal(s) * 0.05)(D, D)),
        "b": _w((lambda *s: _rng.normal(s) * 0.05)(D)),
    }

def reference(x, w, b):
    B, S, D = x.shape
    N, M = 2, 4
    G = D // M
    wg = w.reshape(G, M, D)
    mag = jnp.abs(wg)
    order = jnp.argsort(mag, 1)
    thr = jnp.take_along_axis(mag, order[:, M - N:M - N + 1, :], 1)
    mask = (lambda x, dt: x.astype(dt))(mag >= thr, w.dtype)
    wp = (wg * mask).reshape(D, D)
    return jnp.einsum("bsd,df->bsf", x, wp) + b
```

```python
import functools
import jax
import jax.numpy as jnp
from jax import lax
import jax.experimental.pallas as pl
import jax.experimental.pallas.tpu as pltpu

F32, BF16, I32 = jnp.float32, jnp.bfloat16, jnp.int32

PASSES = {
    "G0": [(96, {(0, 0): 1, (1, 128): 1}, {(0, 0): 1, (128, 1): 1}),
           (32, {(0, 352): 1, (1, 480): -1}, {(352, 0): 1, (480, 1): -1})],
    "G1": [(96, {(0, 256): 1, (1, 384): 1}, {(256, 1): 1, (384, 0): -1}),
           (32, {(0, 96): 1, (1, 224): -1}, {(96, 1): 1, (224, 0): 1})],
    "D00": [(96, {(0, 128): 1, (1, 128): -1}, {(128, 0): 1, (128, 1): 1}),
            (32, {(0, 480): 1, (1, 480): 1}, {(480, 0): 1, (480, 1): -1})],
    "D11": [(96, {(1, 0): 1, (0, 0): -1}, {(0, 0): 1, (0, 1): 1}),
            (32, {(1, 352): 1, (0, 352): 1}, {(352, 1): 1, (352, 0): -1})],
    "D10": [(96, {(0, 256): 1, (1, 256): -1}, {(256, 1): 1, (256, 0): -1}),
            (32, {(1, 96): 1, (0, 96): 1}, {(96, 1): 1, (96, 0): 1})],
    "D01": [(96, {(0, 384): 1, (1, 384): -1}, {(384, 1): 1, (384, 0): -1}),
            (32, {(0, 224): 1, (1, 224): 1}, {(224, 1): 1, (224, 0): 1})],
    "R0p": [(96, {(0, 256): 1, (0, 384): 1}, {(384, 0): 1}),
            (32, {(0, 352): 1, (0, 480): 1}, {(480, 1): 1})],
    "R1p": [(96, {(1, 256): 1, (1, 384): 1}, {(256, 1): 1}),
            (32, {(1, 352): 1, (1, 480): 1}, {(352, 0): 1})],
    "R0m": [(96, {(0, 0): -1, (0, 128): -1}, {(128, 1): 1}),
            (32, {(0, 96): 1, (0, 224): 1}, {(224, 0): 1})],
    "R1m": [(96, {(1, 0): 1, (1, 128): 1}, {(0, 0): 1}),
            (32, {(1, 96): -1, (1, 224): -1}, {(96, 1): 1})],
    "K0a": [(96, {(1, 128): 1}, {(128, 0): 1, (0, 0): -1}),
            (32, {(0, 512): 0.5, (1, 512): 0.5}, {(512, 0): 1})],
    "K0b": [(96, {(0, 256): 1}, {(256, 0): 1, (384, 0): -1}),
            (32, {(0, 544): 0.5, (1, 544): 0.5}, {(544, 0): 1})],
    "K1a": [(96, {(0, 0): 1}, {(0, 1): 1, (128, 1): -1}),
            (32, {(0, 512): 0.5, (1, 512): 0.5}, {(512, 1): 1})],
    "K1b": [(96, {(1, 384): 1}, {(384, 1): 1, (256, 1): -1}),
            (32, {(0, 544): 0.5, (1, 544): 0.5}, {(544, 1): 1})],
    "K0m": [(64, {(0, 512): 0.5, (1, 512): -0.5}, {(512, 0): 1}),
            (32, {(0, 96): 1}, {(96, 0): 1, (224, 0): -1}),
            (32, {(1, 480): 1}, {(352, 0): 1, (480, 0): -1})],
    "K1m": [(64, {(0, 512): 0.5, (1, 512): -0.5}, {(512, 1): 1}),
            (32, {(1, 224): 1}, {(96, 1): 1, (224, 1): -1}),
            (32, {(0, 352): 1}, {(352, 1): 1, (480, 1): -1})],
}
NAMES = tuple(PASSES)
UNIT = 256


def _prune_packed(u):
    mate = lax.broadcasted_iota(I32, u.shape, 0) ^ 1
    lo = pltpu.bitcast((u << 16) & 0x7FFFFFFF, F32)
    hi = pltpu.bitcast(u & 0x7FFF0000, F32)
    big, small = jnp.maximum(lo, hi), jnp.minimum(lo, hi)
    nbig = jnp.take_along_axis(big, mate, axis=0, mode="promise_in_bounds")
    nsmall = jnp.take_along_axis(small, mate, axis=0, mode="promise_in_bounds")
    thr = jnp.maximum(jnp.minimum(big, nbig), jnp.maximum(small, nsmall))
    return u & (jnp.where(lo < thr, 0, 0xFFFF) | jnp.where(hi < thr, 0, -65536))


def _prune_rows(w_bf16):
    u = pltpu.bitcast(w_bf16, I32)
    return [_prune_packed(u[8 * i:8 * i + 8]) for i in range(u.shape[0] // 8)]


def _split(total, sizes):
    assert sum(sizes) == total
    return [(sum(sizes[:j]), sizes[j]) for j in range(len(sizes))]


def _prepare_weights(wbuf, bbuf, wops, bias_ref):
    D, F = wbuf.shape
    H = F // 2
    tiles = []
    for k0 in range(0, 512, 128):
        wp = pltpu.bitcast(jnp.concatenate(_prune_rows(wbuf[k0:k0 + 128, :]), axis=0), BF16)
        tiles.append(wp.T)
    tail = pltpu.bitcast(jnp.concatenate(_prune_rows(wbuf[512:D, :]), axis=0), BF16)
    bias = jnp.broadcast_to(bbuf[...].reshape(1, F).astype(F32), (64, F)).astype(BF16)
    tiles.append(jnp.concatenate([tail, bias], axis=0).T)
    tiles = [t.astype(F32) for t in tiles]
    lane = lax.broadcasted_iota(I32, (H, 128), 1)
    lane2 = lax.broadcasted_iota(I32, (F, 128), 1)
    bias_ref[...] = jnp.where(lane2 < 64, pltpu.roll(tiles[4], 64, 1), tiles[4])
    for p, nm in enumerate(NAMES):
        pos, res = 0, None
        for h, a, _ in PASSES[nm]:
            v = None
            for (i, o), c in sorted(a.items(), key=lambda kv: -kv[1]):
                t = tiles[o // 128][i * H:(i + 1) * H]
                if v is None:
                    v, s = t, c
                else:
                    v = v + t if c == s else v - t
                off = o % 128
            if s != 1:
                v = v * s
            if off != pos:
                v = pltpu.roll(v, (pos - off) % 128, 1)
            res = v if res is None else jnp.where(lane < pos, res, v)
            pos += h
        wops[p] = pltpu.bitcast(res.astype(BF16), I32)


def _unit(wops, bias_ref, xload, ostore):
    H = bias_ref.shape[0] // 2

    def mm(nm):
        parts = []
        for h, _, b in PASSES[nm]:
            items = list(b.items())
            if len(items) == 1:
                parts.append(xload(h, *items[0][0]))
            else:
                p, q = (xload(h, *k).astype(F32) for k, _ in items)
                parts.append((p + q if items[1][1] > 0 else p - q).astype(BF16))
        return jnp.dot(pltpu.bitcast(wops[NAMES.index(nm)], BF16),
                       jnp.concatenate(parts, axis=0), preferred_element_type=F32)

    k = mm("K0a") + mm("K0b"); km = mm("K0m"); d = mm("D00")
    c00 = (k + km) + d; c10 = k - km
    k = mm("K1a") + mm("K1b"); km = mm("K1m"); d = mm("D01")
    c01 = (k + km) + d; c11 = k - km
    rp = mm("R0p") + bias_ref[0:H, :]; rm = mm("R0m"); g0 = mm("G0"); g1 = mm("G1")
    o0 = ((rp + rm) + g0) + c00; o1 = ((rp - rm) + g1) + c01
    ostore(0, jnp.concatenate([o0, o1], axis=1).astype(BF16))
    c10 = c10 - g1; c11 = c11 + g0
    rp = mm("R1p") + bias_ref[H:, :]; rm = mm("R1m"); d0 = mm("D10"); d1 = mm("D11")
    o0 = ((rp + rm) + d0) + c10; o1 = ((rp - rm) + d1) + c11
    ostore(H, jnp.concatenate([o0, o1], axis=1).astype(BF16))


def _kernel(x_hbm, w_hbm, b_hbm, o_hbm, xbuf, obuf, wbuf, bbuf, wops, bias_ref, isem, osem, wsem,
            *, in_split, mode):
    NB, D, S = x_hbm.shape
    RB = obuf.shape[0]
    H = D // 2
    chunks = _split(S, in_split)
    NC = len(chunks)

    def icopy(t, j):
        o, n = chunks[j]
        return pltpu.make_async_copy(
            x_hbm.at[t, :, pl.ds(o, n)], xbuf.at[t, :, pl.ds(o, n)], isem.at[t * NC + j])

    def ocopy(t, slot, o):
        return pltpu.make_async_copy(
            obuf.at[slot, :, pl.ds(o, UNIT)], o_hbm.at[t, :, pl.ds(o, UNIT)], osem.at[slot])

    def owait(slot):
        pltpu.make_async_copy(obuf.at[slot], obuf.at[slot], osem.at[slot]).wait()

    bcp = pltpu.make_async_copy(b_hbm, bbuf, wsem.at[0])
    wcp = pltpu.make_async_copy(w_hbm, wbuf, wsem.at[1])
    wcp.start()
    bcp.start()
    for t in range(NB):
        for j in range(NC):
            icopy(t, j).start()
    bcp.wait()
    wcp.wait()
    _prepare_weights(wbuf, bbuf, wops, bias_ref)

    def wrap(t):
        return jnp.where(t >= RB, t - RB, t)

    def body(t, carry):
        slot = wrap(t)
        writing = t >= NB // 2
        ta = jnp.maximum(2 * t - NB, 0)
        tb = ta + 1
        sa, sb = wrap(ta), wrap(tb)

        if mode != "nowrite":
            @pl.when(t >= RB)
            def _():
                owait(slot)

            @pl.when(writing)
            def _():
                for o in range(0, S, UNIT):
                    ocopy(ta, sa, o).start()

        for o in range(0, S, UNIT):
            for j, (c0, _) in enumerate(chunks):
                if c0 == o:
                    icopy(t, j).wait()

            def xload(h, k0, j):
                return xbuf[t, k0:k0 + h, o + j * 128:o + (j + 1) * 128]

            def ostore(f0, v):
                obuf[slot, f0:f0 + H, o:o + UNIT] = v

            _unit(wops, bias_ref, xload, ostore)

            if mode != "nowrite":
                @pl.when(writing)
                def _():
                    ocopy(tb, sb, o).start()
        return carry

    lax.fori_loop(0, NB, body, 0)
    if mode != "nowrite":
        for s in range(RB):
            owait((NB - RB + s) % RB)


@jax.jit
def pallas_standalone__structured_sparse_n_m__ragged_kernel(
    x: jax.Array,
    w: jax.Array,
    b: jax.Array,
):
    in_split, RB = (512, 1024, 2560), 9
    B, S, D = x.shape
    F = w.shape[1]
    xt = jnp.transpose(x, (0, 2, 1))
    out = pl.pallas_call(
        functools.partial(_kernel, in_split=in_split, mode=""),
        in_specs=[pl.BlockSpec(memory_space=pl.ANY)] * 3,
        out_specs=pl.BlockSpec(memory_space=pl.ANY),
        out_shape=jax.ShapeDtypeStruct((B, F, S), x.dtype),
        scratch_shapes=[
            pltpu.VMEM((B, D, S), x.dtype),
            pltpu.VMEM((RB, F, S), x.dtype),
            pltpu.VMEM((D, F), w.dtype),
            pltpu.VMEM((F,), b.dtype),
            pltpu.VMEM((len(NAMES), F // 4, 128), I32),
            pltpu.VMEM((F, 128), F32),
            pltpu.SemaphoreType.DMA((B * len(in_split),)),
            pltpu.SemaphoreType.DMA((RB,)),
            pltpu.SemaphoreType.DMA((2,)),
        ],
        compiler_params=pltpu.CompilerParams(
            vmem_limit_bytes=124 * 1024 * 1024,
            flags={"XLA_TPU_RESCHEDULE_DMA_DONES": True},
        ),
    )(xt, w, b)
    return jnp.transpose(out, (0, 2, 1))
```

```python
import functools, contextlib
import jax
import jax.numpy as jnp
from jax import lax
import jax.experimental.pallas as pl
import jax.experimental.pallas.tpu as pltpu

F32, BF16, I32 = jnp.float32, jnp.bfloat16, jnp.int32

PASSES = {
    "G0": [(96, {(0, 0): 1, (1, 128): 1}, {(0, 0): 1, (128, 1): 1}),
           (32, {(0, 352): 1, (1, 480): -1}, {(352, 0): 1, (480, 1): -1})],
    "G1": [(96, {(0, 256): 1, (1, 384): 1}, {(256, 1): 1, (384, 0): -1}),
           (32, {(0, 96): 1, (1, 224): -1}, {(96, 1): 1, (224, 0): 1})],
    "D00": [(96, {(0, 128): 1, (1, 128): -1}, {(128, 0): 1, (128, 1): 1}),
            (32, {(0, 480): 1, (1, 480): 1}, {(480, 0): 1, (480, 1): -1})],
    "D11": [(96, {(1, 0): 1, (0, 0): -1}, {(0, 0): 1, (0, 1): 1}),
            (32, {(1, 352): 1, (0, 352): 1}, {(352, 1): 1, (352, 0): -1})],
    "D10": [(96, {(0, 256): 1, (1, 256): -1}, {(256, 1): 1, (256, 0): -1}),
            (32, {(1, 96): 1, (0, 96): 1}, {(96, 1): 1, (96, 0): 1})],
    "D01": [(96, {(0, 384): 1, (1, 384): -1}, {(384, 1): 1, (384, 0): -1}),
            (32, {(0, 224): 1, (1, 224): 1}, {(224, 1): 1, (224, 0): 1})],
    "R0p": [(96, {(0, 256): 1, (0, 384): 1}, {(384, 0): 1}),
            (32, {(0, 352): 1, (0, 480): 1}, {(480, 1): 1})],
    "R1p": [(96, {(1, 256): 1, (1, 384): 1}, {(256, 1): 1}),
            (32, {(1, 352): 1, (1, 480): 1}, {(352, 0): 1})],
    "R0m": [(96, {(0, 0): -1, (0, 128): -1}, {(128, 1): 1}),
            (32, {(0, 96): 1, (0, 224): 1}, {(224, 0): 1})],
    "R1m": [(96, {(1, 0): 1, (1, 128): 1}, {(0, 0): 1}),
            (32, {(1, 96): -1, (1, 224): -1}, {(96, 1): 1})],
    "K0a": [(96, {(1, 128): 1}, {(128, 0): 1, (0, 0): -1}),
            (32, {(0, 512): 0.5, (1, 512): 0.5}, {(512, 0): 1})],
    "K0b": [(96, {(0, 256): 1}, {(256, 0): 1, (384, 0): -1}),
            (32, {(0, 544): 0.5, (1, 544): 0.5}, {(544, 0): 1})],
    "K1a": [(96, {(0, 0): 1}, {(0, 1): 1, (128, 1): -1}),
            (32, {(0, 512): 0.5, (1, 512): 0.5}, {(512, 1): 1})],
    "K1b": [(96, {(1, 384): 1}, {(384, 1): 1, (256, 1): -1}),
            (32, {(0, 544): 0.5, (1, 544): 0.5}, {(544, 1): 1})],
    "K0m": [(64, {(0, 512): 0.5, (1, 512): -0.5}, {(512, 0): 1}),
            (32, {(0, 96): 1}, {(96, 0): 1, (224, 0): -1}),
            (32, {(1, 480): 1}, {(352, 0): 1, (480, 0): -1})],
    "K1m": [(64, {(0, 512): 0.5, (1, 512): -0.5}, {(512, 1): 1}),
            (32, {(1, 224): 1}, {(96, 1): 1, (224, 1): -1}),
            (32, {(0, 352): 1}, {(352, 1): 1, (480, 1): -1})],
}


def _prune_packed(u):
    mate = lax.broadcasted_iota(I32, u.shape, 0) ^ 1
    lo = pltpu.bitcast((u << 16) & 0x7FFFFFFF, F32)
    hi = pltpu.bitcast(u & 0x7FFF0000, F32)
    big, small = jnp.maximum(lo, hi), jnp.minimum(lo, hi)
    nbig = jnp.take_along_axis(big, mate, axis=0, mode="promise_in_bounds")
    nsmall = jnp.take_along_axis(small, mate, axis=0, mode="promise_in_bounds")
    thr = jnp.maximum(jnp.minimum(big, nbig), jnp.maximum(small, nsmall))
    return u & (jnp.where(lo < thr, 0, 0xFFFF) | jnp.where(hi < thr, 0, -65536))


def _prune_rows(w_bf16):
    u = pltpu.bitcast(w_bf16, I32)
    return [_prune_packed(u[8 * i:8 * i + 8]) for i in range(u.shape[0] // 8)]


def _split(total, sizes):
    assert sum(sizes) == total
    return [(sum(sizes[:j]), sizes[j]) for j in range(len(sizes))]


FULL = tuple(n for n in PASSES if n[2:] not in ("a", "b"))
PAIR = 512
G = 64


def _prepare_weights(wbuf, bbuf, wops, wk, bias_ref):
    D, F = wbuf.shape
    H = F // 2
    Q = H // 2
    tiles = []
    for k0 in range(0, 512, 128):
        wp = pltpu.bitcast(jnp.concatenate(_prune_rows(wbuf[k0:k0 + 128, :]), axis=0), BF16)
        tiles.append(wp.T)
    tail = pltpu.bitcast(jnp.concatenate(_prune_rows(wbuf[512:D, :]), axis=0), BF16)
    bias = jnp.broadcast_to(bbuf[...].reshape(1, F).astype(F32), (64, F)).astype(BF16)
    tiles.append(jnp.concatenate([tail, bias], axis=0).T)
    tiles = [t.astype(F32) for t in tiles]
    lane = lax.broadcasted_iota(I32, (H, 128), 1)
    lane2 = lax.broadcasted_iota(I32, (F, 128), 1)
    bias_ref[...] = jnp.where(lane2 < 64, pltpu.roll(tiles[4], 64, 1), tiles[4])

    def operand(nm):
        pos, res = 0, None
        for h, a, _ in PASSES[nm]:
            v = None
            for (i, o), c in sorted(a.items(), key=lambda kv: -kv[1]):
                t = tiles[o // 128][i * H:(i + 1) * H]
                if v is None:
                    v, s = t, c
                else:
                    v = v + t if c == s else v - t
                off = o % 128
            if s != 1:
                v = v * s
            if off != pos:
                v = pltpu.roll(v, (pos - off) % 128, 1)
            res = v if res is None else jnp.where(lane < pos, res, v)
            pos += h
        return res

    for j in range(2):
        a, b = operand("K%da" % j), operand("K%db" % j)
        a0, a1, b0, b1 = a[:Q], a[Q:], b[:Q], b[Q:]
        for i, v in enumerate((a0 + b1, a1 + b1, a0, b1, a0 + b0, a1 - a0, b0 - b1)):
            wk[7 * j + i] = pltpu.bitcast(v.astype(BF16), I32)
    for p, nm in enumerate(FULL):
        wops[p] = pltpu.bitcast(operand(nm).astype(BF16), I32)


def _pair(wops, wk, bias_ref, xload, ostore, tick):
    H = bias_ref.shape[0] // 2

    def xparts(nm, u):
        parts = []
        for h, _, b in PASSES[nm]:
            items = list(b.items())
            if len(items) == 1:
                parts.append(xload(u, h, *items[0][0]))
            else:
                p, q = (xload(u, h, *k).astype(F32) for k, _ in items)
                parts.append(p + q if items[1][1] > 0 else p - q)
        return parts

    def dot(w, parts):
        x = jnp.concatenate([p.astype(BF16) for p in parts], axis=0)
        return jnp.dot(pltpu.bitcast(w, BF16), x, preferred_element_type=F32)

    def mm(nm, u):
        tick(2)
        return dot(wops[FULL.index(nm)], xparts(nm, u))

    def kstr(j):
        a, b = "K%da" % j, "K%db" % j

        def m(i, p, sign=0, q=None):
            tick(1)
            parts = xparts(*p)
            if q is not None:
                parts = [x.astype(F32) + y.astype(F32) if sign > 0 else x.astype(F32) - y.astype(F32)
                         for x, y in zip(parts, xparts(*q))]
            return dot(wk[7 * j + i], parts)

        m2 = m(1, (a, 0))
        m4 = m(3, (b, 0), -1, (a, 0))
        m1 = m(0, (a, 0), 1, (b, 1))
        m7 = m(6, (b, 0), 1, (b, 1))
        c10 = m2 + m4; t00 = (m1 + m4) + m7; t11 = m1 - m2
        m5 = m(4, (b, 1))
        m3 = m(2, (a, 1), -1, (b, 1))
        m6 = m(5, (a, 0), 1, (a, 1))
        c00 = t00 - m5; c01 = m3 + m5; c11 = (m3 + m6) + t11
        return jnp.concatenate([c00, c10], axis=0), jnp.concatenate([c01, c11], axis=0)

    k0 = kstr(0)
    k1 = kstr(1)
    for u in range(2):
        km0 = mm("K0m", u); d0 = mm("D00", u); km1 = mm("K1m", u); d1 = mm("D01", u)
        c00 = (km0 + d0) + k0[u]; c10 = k0[u] - km0
        c01 = (km1 + d1) + k1[u]; c11 = k1[u] - km1
        rp = mm("R0p", u) + bias_ref[0:H, :]; rm = mm("R0m", u); g0 = mm("G0", u); g1 = mm("G1", u)
        o0 = ((rp + rm) + g0) + c00; o1 = ((rp - rm) + g1) + c01
        ostore(u, 0, jnp.concatenate([o0, o1], axis=1).astype(BF16))
        c10 = c10 - g1; c11 = c11 + g0
        rp = mm("R1p", u) + bias_ref[H:, :]; rm = mm("R1m", u); d0 = mm("D10", u); d1 = mm("D11", u)
        o0 = ((rp + rm) + d0) + c10; o1 = ((rp - rm) + d1) + c11
        ostore(u, H, jnp.concatenate([o0, o1], axis=1).astype(BF16))


def _kernel(x_hbm, w_hbm, b_hbm, o_hbm, xbuf, obuf, wbuf, bbuf, wops, wk, bias_ref, isem, osem, wsem,
            *, in_split, nchunked, pos, skip, lead, last, wch, mode):
    D = w_hbm.shape[0]
    S = x_hbm.shape[1]
    NB = x_hbm.shape[0] // D
    NG = D // G
    RB = obuf.shape[0] // NG
    H = D // 2
    chunks = _split(S, in_split)
    NP = len(pos) * (S // PAIR)
    NC = len(chunks)
    npaced = NP * (NB // 2) - skip
    assert npaced % 2 == 0
    bulk_end = NB * D - npaced * 4

    def chunk_copy(t, j):
        o, n = chunks[j]
        idx = (pl.ds(t * D, D), pl.ds(o, n))
        return pltpu.make_async_copy(x_hbm.at[idx], xbuf.at[idx], isem.at[NB + t * NC + j])

    def batch_wait(t):
        v = xbuf.at[pl.ds(pl.multiple_of(t * D, D), D)]
        pltpu.make_async_copy(v, v, isem.at[t]).wait()

    bcp = pltpu.make_async_copy(b_hbm, bbuf, wsem.at[0])
    wcp = pltpu.make_async_copy(w_hbm, wbuf, wsem.at[1])
    wcp.start()
    bcp.start()
    for t in range(nchunked):
        for j in range(NC):
            chunk_copy(t, j).start(priority=1)
    for t in range(nchunked, NB):
        n = min(D, bulk_end - t * D)
        if n > 0:
            pltpu.make_async_copy(x_hbm.at[pl.ds(t * D, n)], xbuf.at[pl.ds(t * D, n)],
                                  isem.at[t]).start(priority=1)
    scope = jax.named_scope if mode == "prof" else (lambda n: contextlib.nullcontext())
    with scope("wwait"):
        bcp.wait()
        wcp.wait()
    with scope("prep"):
        _prepare_weights(wbuf, bbuf, wops, wk, bias_ref)

    def wrap(t):
        return jnp.where(t >= RB, t - RB, t)

    def owait(slot, nb):
        v = obuf.at[pl.ds(slot * NG, nb * NG)]
        pltpu.make_async_copy(v, v, osem.at[slot]).wait()

    def ocopy(t, slot, nb, r0, nr, c0, nc, g0=0, ng=NG):
        n = ng if nb == 1 else nb * NG
        return pltpu.make_async_copy(
            obuf.at[pl.ds(slot * NG + g0, n), pl.ds(r0, nr), pl.ds(c0, nc)],
            o_hbm.at[pl.ds(t * NG + g0, n), pl.ds(r0, nr), pl.ds(c0, nc)], osem.at[slot])

    wdescs = [(r0, c0) for r0 in range(0, G, 8) for c0 in range(0, S, wch)]
    NW = len(wdescs)
    HALF = NB // 2
    TICKS = 62 * (S // PAIR)
    NST = 4 * (S // PAIR)

    def body(t, carry):
        slot = wrap(t)
        row0 = pl.multiple_of(t * D, D)
        state = {"tick": 0, "paced": 0, "stores": 0, "w": 0, "l": 0}

        @pl.when((t >= RB) & ((t & 1) == 0))
        def _():
            owait(slot, 2)

        @pl.when(t >= nchunked)
        def _():
            batch_wait(t)

        def tick(n):
            if state["tick"] % 62 in pos:
                i = state["paced"]
                q = t * NP + (i - skip)
                r = pl.multiple_of(bulk_end + t * (NP * 4) + ((i - skip) // 2) * 8, 8)
                idx = (pl.ds(r, 8), pl.ds(((i - skip) % 2) * (S // 2), S // 2))
                cond = t < HALF
                if i < skip:
                    cond = cond & (t > 0)

                @pl.when(cond)
                def _():
                    bt = (r * 7282) >> 22
                    pltpu.make_async_copy(x_hbm.at[idx], xbuf.at[idx], isem.at[bt]).start()
                state["paced"] += 1
            state["tick"] += n

        def writes(frac):
            while state["w"] < frac * NW:
                n = state["w"] + lead
                tp = 2 * (t - HALF + n // NW)
                r0, c0 = wdescs[n % NW]

                @pl.when((tp >= 0) & (tp < NB - 2))
                def _():
                    ocopy(tp, wrap(tp), 2, r0, 8, c0, wch).start()
                state["w"] += 1
            while state["l"] < min(NW, 2 * (frac * NW + lead)):
                r0, c0 = wdescs[state["l"]]

                @pl.when(t == NB - 1)
                def _():
                    ocopy(NB - 2, (NB - 2) % RB, 1, r0, 8, c0, wch).start()
                state["l"] += 1

        fr = [(14 + 24 * u + 16 + 8 * k) / 62 for u in range(2) for k in range(2)]
        npair = S // PAIR
        lasts = _split(S, last)
        pending = []
        writes(fr[0] / npair)
        for p in range(npair):
            o = p * PAIR
            for j, (c0, _) in enumerate(chunks):
                if c0 == o:
                    @pl.when(t < nchunked)
                    def _():
                        idx = (pl.ds(row0, D), pl.ds(c0, chunks[j][1]))
                        pltpu.make_async_copy(xbuf.at[idx], xbuf.at[idx], isem.at[NB + t * NC + j]).wait()

            def xload(u, h, k0, j):
                c = o + u * 256 + j * 128
                return xbuf[pl.ds(row0 + k0, h), c:c + 128]

            def ostore(u, f0, v):
                c = o + u * 256
                f = f0
                while f < f0 + H:
                    g, r = divmod(f, G)
                    n = min(G - r, f0 + H - f)
                    obuf[slot * NG + g, r:r + n, c:c + 256] = v[f - f0:f - f0 + n]
                    f += n
                k = state["stores"] = state["stores"] + 1
                if k < NST:
                    writes((k // 4 + fr[k % 4]) / npair)
                if f0:
                    for c0, n in lasts:
                        if c0 + n == c + 256:
                            if n >= 1024:
                                ds = [(r0, 8, cc, 512) for r0 in range(0, G, 8) for cc in range(c0, c0 + n, 512)]
                            else:
                                ds = [(0, G, cc, 256) for cc in range(c0, c0 + n, 256)]
                            pending.extend(ds)
                for _ in range(len(pending) if k == NST else min(8, len(pending))):
                    d = pending.pop(0)

                    @pl.when(t == NB - 1)
                    def _():
                        ocopy(NB - 1, (NB - 1) % RB, 1, *d).start()

            _pair(wops, wk, bias_ref, xload, ostore, tick)
        return carry

    def sbody(t, c):
        with scope("iter"):
            return body(t, c)

    lax.fori_loop(0, NB, sbody, 0)
    with scope("tail"):
        for t in range(NB - RB, NB - 2, 2):
            owait(t % RB, 2)
        owait((NB - 2) % RB, 1)
        owait((NB - 1) % RB, 1)


def make(in_split=(512, 512, 1024, 1024, 1024), nchunked=2, pos=(0, 7, 14, 22, 30, 38, 46, 54), skip=0, lead=6,
         last=(2048,) + (256,) * 8, wch=512, RB=10,
         flags=("XLA_TPU_RESCHEDULE_DMA_DONES",), mode=""):
    def fn(x, w, b):
        B, S, D = x.shape
        F = w.shape[1]
        xt = jnp.transpose(x, (0, 2, 1)).reshape(B * D, S)
        out = pl.pallas_call(
            functools.partial(_kernel, in_split=in_split, nchunked=nchunked, pos=pos, skip=skip, lead=lead,
                              last=last, wch=wch, mode=mode),
            in_specs=[pl.BlockSpec(memory_space=pl.ANY)] * 3,
            out_specs=pl.BlockSpec(memory_space=pl.ANY),
            out_shape=jax.ShapeDtypeStruct((B * F // G, G, S), x.dtype),
            scratch_shapes=[
                pltpu.VMEM((B * D, S), x.dtype),
                pltpu.VMEM((RB * F // G, G, S), x.dtype),
                pltpu.VMEM((D, F), w.dtype),
                pltpu.VMEM((F,), b.dtype),
                pltpu.VMEM((len(FULL), F // 4, 128), I32),
                pltpu.VMEM((14, F // 8, 128), I32),
                pltpu.VMEM((F, 128), F32),
                pltpu.SemaphoreType.DMA((B + nchunked * len(in_split),)),
                pltpu.SemaphoreType.DMA((RB,)),
                pltpu.SemaphoreType.DMA((2,)),
            ],
            compiler_params=pltpu.CompilerParams(
                vmem_limit_bytes=127 * 1024 * 1024,
                flags={k: True for k in flags} or None,
                disable_bounds_checks=True,
                disable_semaphore_checks=True,
            ),
            name="k2",
        )(xt, w, b)
        return jnp.transpose(out.reshape(B, F, S), (0, 2, 1))
    return fn


@jax.jit
def pallas_standalone__structured_sparse_n_m__ragged_kernel(
    x: jax.Array,
    w: jax.Array,
    b: jax.Array,
):
    return make(lead=12)(x, w, b)
```

```python
import functools, contextlib
import jax
import jax.numpy as jnp
from jax import lax
import jax.experimental.pallas as pl
import jax.experimental.pallas.tpu as pltpu

F32, BF16, I32 = jnp.float32, jnp.bfloat16, jnp.int32


def _prune_packed(u):
    mate = lax.broadcasted_iota(I32, u.shape, 0) ^ 1
    lo = pltpu.bitcast((u << 16) & 0x7FFFFFFF, F32)
    hi = pltpu.bitcast(u & 0x7FFF0000, F32)
    big, small = jnp.maximum(lo, hi), jnp.minimum(lo, hi)
    nbig = jnp.take_along_axis(big, mate, axis=0, mode="promise_in_bounds")
    nsmall = jnp.take_along_axis(small, mate, axis=0, mode="promise_in_bounds")
    thr = jnp.maximum(jnp.minimum(big, nbig), jnp.maximum(small, nsmall))
    return u & (jnp.where(lo < thr, 0, 0xFFFF) | jnp.where(hi < thr, 0, -65536))


def _prune_rows(w_bf16):
    u = pltpu.bitcast(w_bf16, I32)
    return [_prune_packed(u[8 * i:8 * i + 8]) for i in range(u.shape[0] // 8)]


def _split(total, sizes):
    assert sum(sizes) == total
    return [(sum(sizes[:j]), sizes[j]) for j in range(len(sizes))]


PASSES = {
    "Gp": [(96, {(0, 0): 1, (1, 128): 1}, {(0, 0): 1, (128, 1): 1}),
           (32, {(0, 352): 1, (1, 480): -1}, {(352, 0): 1, (480, 1): -1})],
    "Gm": [(96, {(0, 256): 1, (1, 384): 1}, {(256, 0): 1, (384, 1): -1}),
           (32, {(0, 96): 1, (1, 224): -1}, {(96, 0): 1, (224, 1): 1})],
    "R0p": [(96, {(0, 256): 1, (0, 384): 1}, {(384, 1): 1}),
            (32, {(0, 352): 1, (0, 480): 1}, {(480, 1): 1})],
    "R1p": [(96, {(1, 256): 1, (1, 384): 1}, {(256, 0): 1}),
            (32, {(1, 352): 1, (1, 480): 1}, {(352, 0): 1})],
    "R0n": [(96, {(0, 0): 1, (0, 128): 1}, {(128, 1): 1}),
            (32, {(0, 96): 1, (0, 224): 1}, {(224, 1): 1})],
    "R1m": [(96, {(1, 0): 1, (1, 128): 1}, {(0, 0): 1}),
            (32, {(1, 96): 1, (1, 224): 1}, {(96, 0): 1})],
    "K0m": [(64, {(0, 512): 0.5, (1, 512): -0.5}, {(512, 0): 1}),
            (32, {(1, 224): 1}, {(96, 0): 1, (224, 0): -1}),
            (32, {(1, 480): 1}, {(352, 0): 1, (480, 0): -1})],
    "K1m": [(64, {(0, 512): 0.5, (1, 512): -0.5}, {(512, 1): 1}),
            (32, {(0, 96): 1}, {(96, 1): 1, (224, 1): -1}),
            (32, {(0, 352): 1}, {(352, 1): 1, (480, 1): -1})],
    "K0a": [(96, {(1, 128): 1}, {(128, 0): 1, (0, 0): -1}),
            (32, {(0, 512): 0.5, (1, 512): 0.5}, {(512, 0): 1})],
    "K0b": [(96, {(1, 384): 1}, {(384, 0): 1, (256, 0): -1}),
            (32, {(0, 544): 0.5, (1, 544): 0.5}, {(544, 0): 1})],
    "K1a": [(96, {(0, 0): 1}, {(0, 1): 1, (128, 1): -1}),
            (32, {(0, 512): 0.5, (1, 512): 0.5}, {(512, 1): 1})],
    "K1b": [(96, {(0, 256): 1}, {(256, 1): 1, (384, 1): -1}),
            (32, {(0, 544): 0.5, (1, 544): 0.5}, {(544, 1): 1})],
    "D0a": [(96, {(0, 128): 1, (1, 128): -1}, {(128, 0): 1, (128, 1): 1}),
            (32, {(0, 224): 1, (1, 224): 1}, {(224, 0): 1, (224, 1): 1})],
    "D0b": [(96, {(0, 384): 1, (1, 384): -1}, {(384, 0): 1, (384, 1): -1}),
            (32, {(0, 480): 1, (1, 480): 1}, {(480, 0): 1, (480, 1): -1})],
    "D1a": [(96, {(1, 0): 1, (0, 0): -1}, {(0, 0): 1, (0, 1): 1}),
            (32, {(1, 96): 1, (0, 96): 1}, {(96, 0): 1, (96, 1): 1})],
    "D1b": [(96, {(0, 256): 1, (1, 256): -1}, {(256, 0): 1, (256, 1): -1}),
            (32, {(1, 352): -1, (0, 352): -1}, {(352, 0): 1, (352, 1): -1})],
}
FULL = tuple(n for n in PASSES if n[2:] not in ("a", "b"))
DOUBLE = ("K0", "K1", "D0", "D1")
TICKS = 60


def prepare_weights(wbuf, bbuf, wops, wk, bias_ref):
    D, F = wbuf.shape
    H = F // 2
    Q = H // 2
    tiles = []
    for k0 in range(0, 512, 128):
        wp = pltpu.bitcast(jnp.concatenate(_prune_rows(wbuf[k0:k0 + 128, :]), axis=0), BF16)
        tiles.append(wp.T)
    tail = pltpu.bitcast(jnp.concatenate(_prune_rows(wbuf[512:D, :]), axis=0), BF16)
    bias = jnp.broadcast_to(bbuf[...].reshape(1, F).astype(F32), (64, F)).astype(BF16)
    tiles.append(jnp.concatenate([tail, bias], axis=0).T)
    tiles = [t.astype(F32) for t in tiles]
    lane = lax.broadcasted_iota(I32, (H, 128), 1)
    lane2 = lax.broadcasted_iota(I32, (F, 128), 1)
    bias_ref[...] = jnp.where(lane2 < 64, pltpu.roll(tiles[4], 64, 1), tiles[4])

    def operand(nm):
        pos, res = 0, None
        for h, a, _ in PASSES[nm]:
            v = None
            for (i, o), c in sorted(a.items(), key=lambda kv: -kv[1]):
                t = tiles[o // 128][i * H:(i + 1) * H]
                if v is None:
                    v, s = t, c
                else:
                    v = v + t if c == s else v - t
                off = o % 128
            if s != 1:
                v = v * s
            if off != pos:
                v = pltpu.roll(v, (pos - off) % 128, 1)
            res = v if res is None else jnp.where(lane < pos, res, v)
            pos += h
        return res

    for p, nm in enumerate(FULL):
        wops[p] = pltpu.bitcast(operand(nm).astype(BF16), I32)
    for j, nm in enumerate(DOUBLE):
        a, b = operand(nm + "a"), operand(nm + "b")
        a0, a1, b0, b1 = a[:Q], a[Q:], b[:Q], b[Q:]
        for i, v in enumerate((a0 + b1, a1 + b1, a0, b1, a0 + b0, a1 - a0, b0 - b1)):
            wk[7 * j + i] = pltpu.bitcast(v.astype(BF16), I32)


def pair(wops, wk, bias_ref, xload, ostore, tick, order="C"):
    H = bias_ref.shape[0] // 2

    def xparts(nm, u):
        parts = []
        for h, _, b in PASSES[nm]:
            items = list(b.items())
            if len(items) == 1:
                parts.append(xload(u, h, *items[0][0]))
            else:
                p, q = (xload(u, h, *k).astype(F32) for k, _ in items)
                parts.append(p + q if items[1][1] > 0 else p - q)
        return parts

    def dot(w, parts):
        x = jnp.concatenate([p.astype(BF16) for p in parts], axis=0)
        return jnp.dot(pltpu.bitcast(w, BF16), x, preferred_element_type=F32)

    def mm(nm, u):
        tick(2)
        if nm[0] == "R":
            (k0, j), = PASSES[nm][0][2]
            return dot(wops[FULL.index(nm)], [xload(u, 128, k0, j)])
        return dot(wops[FULL.index(nm)], xparts(nm, u))

    def strassen(nm):
        j = DOUBLE.index(nm)
        a, b = nm + "a", nm + "b"

        def m(i, p, sign=0, q=None):
            tick(1)
            parts = xparts(*p)
            if q is not None:
                parts = [x.astype(F32) + y.astype(F32) if sign > 0 else x.astype(F32) - y.astype(F32)
                         for x, y in zip(parts, xparts(*q))]
            return dot(wk[7 * j + i], parts)

        m2 = m(1, (a, 0))
        m4 = m(3, (b, 0), -1, (a, 0))
        m1 = m(0, (a, 0), 1, (b, 1))
        m7 = m(6, (b, 0), 1, (b, 1))
        c10 = m2 + m4; t00 = (m1 + m4) + m7; t11 = m1 - m2
        m5 = m(4, (b, 1))
        m3 = m(2, (a, 1), -1, (b, 1))
        m6 = m(5, (a, 0), 1, (a, 1))
        c00 = t00 - m5; c01 = m3 + m5; c11 = (m3 + m6) + t11
        return jnp.concatenate([c00, c10], axis=0), jnp.concatenate([c01, c11], axis=0)

    def rows(u):
        p0 = mm("R0p", u) + bias_ref[0:H, :]; n0 = mm("R0n", u)
        p1 = mm("R1p", u) + bias_ref[H:, :]; m1 = mm("R1m", u)
        return p0 - n0, p0 + n0, p1 + m1, p1 - m1

    def cols(u, k0, k1, d0, d1):
        gp = mm("Gp", u); gm = mm("Gm", u); m0 = mm("K0m", u); m1 = mm("K1m", u)
        return (((gp + gm) + m0) + (k0[u] + d0[u]), k1[u] + m1, k0[u] - m0,
                ((gp - gm) - m1) + (k1[u] + d1[u]))

    def emit(u, r, c):
        o = [x + y for x, y in zip(c, r)]
        ostore(u, jnp.concatenate(o[:2], axis=1).astype(BF16), jnp.concatenate(o[2:], axis=1).astype(BF16))

    if order == "B":
        s = [strassen(n) for n in DOUBLE]
        for u in range(2):
            c = cols(u, *s)
            emit(u, rows(u), c)
    elif order == "C":
        r = [rows(0), rows(1)]
        s = [strassen(n) for n in DOUBLE]
        for u in range(2):
            emit(u, r[u], cols(u, *s))
    elif order == "D":
        r0 = rows(0)
        s = [strassen(n) for n in DOUBLE]
        emit(0, r0, cols(0, *s))
        c = cols(1, *s)
        emit(1, rows(1), c)
    elif order == "E":
        r0 = rows(0)
        s = [strassen(n) for n in DOUBLE]
        r1 = rows(1)
        emit(0, r0, cols(0, *s))
        emit(1, r1, cols(1, *s))


PAIR = 512
G = 64


def _kernel(x_hbm, w_hbm, b_hbm, o_hbm, xbuf, obuf, wbuf, bbuf, wops, wk, bias_ref, sem, osem,
            *, pos, rlead, stop, lead, last, wch, mode, rdend, order, csem, wpos, burst):
    D = w_hbm.shape[0]
    S = x_hbm.shape[2]
    NG = D // G
    NB = x_hbm.shape[0] // NG
    RB = obuf.shape[0] // NG
    H = D // 2
    HALF = NB // 2
    npair = S // PAIR
    NP = 64
    assert len(pos) * npair == NP
    scope = jax.named_scope if "prof" in mode else (lambda n: contextlib.nullcontext())

    WS = NB + npair

    def icopy(t, r, c, k):
        if not isinstance(r, int):
            r, c = pl.multiple_of(r, 8), pl.multiple_of(c, PAIR)
        idx = (pl.ds(t * NG, NG), pl.ds(r, 8), pl.ds(c, PAIR))
        return pltpu.make_async_copy(x_hbm.at[idx], xbuf.at[idx], sem.at[k])

    first_b = [(0, 8 * r, c * PAIR, NB + csem[c]) for c in range(npair) for r in range(0 if c < 2 else 4, 8)]
    first_b += [(1, 8 * r, c * PAIR, 1) for r in range(5, 8) for c in range(npair)]
    first_a = [(0, 8 * r, c * PAIR, NB + csem[c]) for c in range(2, npair) for r in range(4)]
    first_a += [(1, 8 * r, c * PAIR, 1) for r in range(5) for c in range(npair)]
    piece = [(8 * r, c * PAIR) for r in range(8) for c in range(npair)]

    bcp = pltpu.make_async_copy(b_hbm, bbuf, sem.at[WS])
    wcp = pltpu.make_async_copy(w_hbm, wbuf, sem.at[WS + 1])
    wcp.start()
    bcp.start()
    assert 16 <= rlead <= 40

    def pro(i, c):
        ch = jnp.where(i < 16, i >> 3, (i >> 2) - 2)
        r = jnp.where(i < 16, i & 7, (i & 3) + 4)
        k = NB + ch
        for c0 in range(npair):
            if csem[c0] != c0:
                k = jnp.where(ch == c0, NB + csem[c0], k)
        icopy(0, r * 8, ch * PAIR, k).start(priority=1)
        return c

    lax.fori_loop(0, rlead, pro, 0)
    with scope("wwait"):
        bcp.wait()
        wcp.wait()
    with scope("prep"):
        prepare_weights(wbuf, bbuf, wops, wk, bias_ref)

    def wrap(t):
        return jnp.where(t >= RB, t - RB, t)

    def owait(slot, nb):
        v = obuf.at[pl.ds(slot * NG, nb * NG)]
        pltpu.make_async_copy(v, v, osem.at[slot]).wait()

    def ocopy(t, slot, nb, r0, nr, c0, nc):
        return pltpu.make_async_copy(
            obuf.at[pl.ds(slot * NG, nb * NG), pl.ds(r0, nr), pl.ds(c0, nc)],
            o_hbm.at[pl.ds(t * NG, nb * NG), pl.ds(r0, nr), pl.ds(c0, nc)], osem.at[slot])

    def batch_wait(t):
        v = xbuf.at[pl.ds(t * NG, NG)]
        pltpu.make_async_copy(v, v, sem.at[t]).wait()

    wdescs = [(r0, c0) for r0 in range(0, G, 8) for c0 in range(0, S, wch)]
    NW = len(wdescs)

    lastd = []
    for c0, n in _split(S, last):
        if n >= 1024:
            lastd.append((c0 + n, [(r0, 8, cc, 512) for r0 in range(0, G, 8) for cc in range(c0, c0 + n, 512)]))
        elif n == 512:
            lastd.append((c0 + n, [(r0, 8, c0, 512) for r0 in range(0, G, 8)]))
        else:
            lastd.append((c0 + n, [(0, G, c0, 256)]))
    pending = []

    def body(t, carry):
        slot = wrap(t)
        state = {"tick": 0, "paced": 0, "w": 0, "l": 0}
        first = t == 0

        @pl.when((t >= RB) & ((t & 1) == 0))
        def _():
            owait(slot, 2)

        @pl.when((t > 0) & (t < HALF) if rdend else (t > 0))
        def _():
            batch_wait(t)

        def pick(a, b):
            return [jnp.where(first, p, q) for p, q in zip(a, b)]

        def tick(n):
            q = state["tick"] % TICKS
            for _ in range(wpos.count(q) if n else 0):
                write()
            for _ in range((pos.count(q) if n else pos.count(TICKS))):
                i = state["paced"]
                da = pick(first_a[i], (2 * t + 1, *piece[i], 2 * t + 1))

                @pl.when(t < (HALF if i < NP - stop else HALF - 1))
                def _():
                    icopy(*da).start(priority=0)
                j = i + rlead
                if j < NP:
                    db = pick(first_b[j], (2 * t, *piece[j], 2 * t))

                    @pl.when(t < HALF)
                    def _():
                        icopy(*db).start(priority=1)
                else:
                    @pl.when(t < HALF - 1)
                    def _():
                        icopy(2 * t + 2, *piece[j - NP], 2 * t + 2).start(priority=1)
                    if j - NP < stop:
                        @pl.when(t == HALF - 1)
                        def _():
                            icopy(NB - 1, *piece[j - stop], NB - 1).start(priority=1)
                state["paced"] += 1
            state["tick"] += n

        def write():
            i = state["w"]
            n = i + lead + burst
            tp = 2 * (t - HALF + n // NW)
            if i == NW - lead:
                for r0, c0 in wdescs[:burst]:
                    @pl.when(t == HALF - 1)
                    def _():
                        ocopy(0, 0, 2, r0, 8, c0, wch).start()
            r0, c0 = wdescs[n % NW]
            lo = 2 if n >= NW and i < NW - lead else 0

            @pl.when((tp >= lo) & (tp < NB - 2))
            def _():
                ocopy(tp, wrap(tp), 2, r0, 8, c0, wch).start()
            state["w"] += 1
            while state["l"] < min(NW, 2 * (i + 1 + lead + burst)):
                r0, c0 = wdescs[state["l"]]

                @pl.when(t == NB - 1)
                def _():
                    ocopy(NB - 2, (NB - 2) % RB, 1, r0, 8, c0, wch).start()
                state["l"] += 1
            for _ in range(min(2, len(pending))):
                d = pending.pop(0)

                @pl.when(t == NB - 1)
                def _():
                    ocopy(NB - 1, (NB - 1) % RB, 1, *d).start()

        for p in range(npair):
            o = p * PAIR
            if rdend and p == rdend:
                @pl.when(t == HALF - 1)
                def _():
                    with scope("rdwait"):
                        for q in range(HALF, NB):
                            batch_wait(q)

            if csem[p] == p:
                @pl.when(first)
                def _():
                    v = xbuf.at[pl.ds(0, NG), :, pl.ds(o, PAIR * csem.count(p))]
                    pltpu.make_async_copy(v, v, sem.at[NB + p]).wait()

            def xload(u, h, k0, j):
                c = o + u * 256 + j * 128
                parts, k = [], k0
                while k < k0 + h:
                    g, r = divmod(k, G)
                    n = min(G - r, k0 + h - k)
                    parts.append(xbuf[t * NG + g, r:r + n, c:c + 128])
                    k += n
                return jnp.concatenate(parts, axis=0)

            def ostore(u, v0, v1):
                c = o + u * 256
                if v0 is not None:
                    v = jnp.concatenate([v0, v1], axis=0)
                    for g in range(NG):
                        obuf[slot * NG + g, :, c:c + 256] = v[g * G:(g + 1) * G]
                for end, ds in lastd:
                    if end == c + 256:
                        pending.extend(ds)

            if "nocomp" in mode:
                z = jnp.zeros((H, 256), BF16)
                for q, n in enumerate([8, 8, 8, 4, 8, 8, 8, 8]):
                    tick(n)
                    pl.delay(int(n * 24.1))
                    if q in (5, 7):
                        ostore((q - 5) // 2, None, None)
            else:
                pair(wops, wk, bias_ref, xload, ostore, tick, order)
            tick(0)
        return carry

    def sbody(t, c):
        with scope("iter"):
            return body(t, c)

    lax.fori_loop(0, NB, sbody, 0)
    with scope("tail"):
        for d in pending:
            ocopy(NB - 1, (NB - 1) % RB, 1, *d).start()
        for t in range(NB - RB, NB - 2, 2):
            owait(t % RB, 2)
        owait((NB - 2) % RB, 1)
        owait((NB - 1) % RB, 1)


def make(RB=10, flags=("XLA_TPU_RESCHEDULE_DMA_DONES",), **kw):
    cfg = dict(pos=(0, 8, 16, 24, 28, 36, 44, 52), rlead=20, stop=6, lead=6, last=(2048, 1024, 1024), wch=512,
               mode="", rdend=0, order="B", csem=(0, 1, 2, 3, 4, 4, 6, 6), wpos=(36, 36, 52, 52, 52, 52, 52, 52), burst=2)
    cfg.update(kw)

    def fn(x, w, b):
        B, S, D = x.shape
        F = w.shape[1]
        xt = jnp.transpose(x, (0, 2, 1)).reshape(B * D // G, G, S)
        out = pl.pallas_call(
            functools.partial(_kernel, **cfg),
            in_specs=[pl.BlockSpec(memory_space=pl.ANY)] * 3,
            out_specs=pl.BlockSpec(memory_space=pl.ANY),
            out_shape=jax.ShapeDtypeStruct((B * F // G, G, S), x.dtype),
            scratch_shapes=[
                pltpu.VMEM((B * D // G, G, S), x.dtype),
                pltpu.VMEM((RB * F // G, G, S), x.dtype),
                pltpu.VMEM((D, F), w.dtype),
                pltpu.VMEM((F,), b.dtype),
                pltpu.VMEM((len(FULL), F // 4, 128), I32),
                pltpu.VMEM((28, F // 8, 128), I32),
                pltpu.VMEM((F, 128), F32),
                pltpu.SemaphoreType.DMA((B + S // PAIR + 2,)),
                pltpu.SemaphoreType.DMA((RB,)),
            ],
            compiler_params=pltpu.CompilerParams(
                vmem_limit_bytes=127 * 1024 * 1024,
                flags={k: True for k in flags} or None,
                disable_bounds_checks=True,
                disable_semaphore_checks=True,
            ),
            name="k3",
        )(xt, w, b)
        return jnp.transpose(out.reshape(B, F, S), (0, 2, 1))
    return fn


@jax.jit
def pallas_standalone__structured_sparse_n_m__ragged_kernel(
    x: jax.Array,
    w: jax.Array,
    b: jax.Array,
):
    return make(rlead=24)(x, w, b)
```

```python
import functools, contextlib
import jax
import jax.numpy as jnp
from jax import lax
import jax.experimental.pallas as pl
import jax.experimental.pallas.tpu as pltpu

F32, BF16, I32 = jnp.float32, jnp.bfloat16, jnp.int32


def _prune_packed(u):
    mate = lax.broadcasted_iota(I32, u.shape, 0) ^ 1
    lo = pltpu.bitcast((u << 16) & 0x7FFFFFFF, F32)
    hi = pltpu.bitcast(u & 0x7FFF0000, F32)
    big, small = jnp.maximum(lo, hi), jnp.minimum(lo, hi)
    nbig = jnp.take_along_axis(big, mate, axis=0, mode="promise_in_bounds")
    nsmall = jnp.take_along_axis(small, mate, axis=0, mode="promise_in_bounds")
    thr = jnp.maximum(jnp.minimum(big, nbig), jnp.maximum(small, nsmall))
    return u & (jnp.where(lo < thr, 0, 0xFFFF) | jnp.where(hi < thr, 0, -65536))


def _prune_rows(w_bf16):
    u = pltpu.bitcast(w_bf16, I32)
    return [_prune_packed(u[8 * i:8 * i + 8]) for i in range(u.shape[0] // 8)]


def _split(total, sizes):
    assert sum(sizes) == total
    return [(sum(sizes[:j]), sizes[j]) for j in range(len(sizes))]


PASSES = {
    "Gp": [(96, {(0, 0): 1, (1, 128): 1}, {(0, 0): 1, (128, 1): 1}),
           (32, {(0, 352): 1, (1, 480): -1}, {(352, 0): 1, (480, 1): -1})],
    "Gm": [(96, {(0, 256): 1, (1, 384): 1}, {(256, 0): 1, (384, 1): -1}),
           (32, {(0, 96): 1, (1, 224): -1}, {(96, 0): 1, (224, 1): 1})],
    "R0p": [(96, {(0, 256): 1, (0, 384): 1}, {(384, 1): 1}),
            (32, {(0, 352): 1, (0, 480): 1}, {(480, 1): 1})],
    "R1p": [(96, {(1, 256): 1, (1, 384): 1}, {(256, 0): 1}),
            (32, {(1, 352): 1, (1, 480): 1}, {(352, 0): 1})],
    "R0n": [(96, {(0, 0): 1, (0, 128): 1}, {(128, 1): 1}),
            (32, {(0, 96): 1, (0, 224): 1}, {(224, 1): 1})],
    "R1m": [(96, {(1, 0): 1, (1, 128): 1}, {(0, 0): 1}),
            (32, {(1, 96): 1, (1, 224): 1}, {(96, 0): 1})],
    "K0m": [(64, {(0, 512): 0.5, (1, 512): -0.5}, {(512, 0): 1}),
            (32, {(1, 224): 1}, {(96, 0): 1, (224, 0): -1}),
            (32, {(1, 480): 1}, {(352, 0): 1, (480, 0): -1})],
    "K1m": [(64, {(0, 512): 0.5, (1, 512): -0.5}, {(512, 1): 1}),
            (32, {(0, 96): 1}, {(96, 1): 1, (224, 1): -1}),
            (32, {(0, 352): 1}, {(352, 1): 1, (480, 1): -1})],
    "K0a": [(96, {(1, 128): 1}, {(128, 0): 1, (0, 0): -1}),
            (32, {(0, 512): 0.5, (1, 512): 0.5}, {(512, 0): 1})],
    "K0b": [(96, {(1, 384): 1}, {(384, 0): 1, (256, 0): -1}),
            (32, {(0, 544): 0.5, (1, 544): 0.5}, {(544, 0): 1})],
    "K1a": [(96, {(0, 0): 1}, {(0, 1): 1, (128, 1): -1}),
            (32, {(0, 512): 0.5, (1, 512): 0.5}, {(512, 1): 1})],
    "K1b": [(96, {(0, 256): 1}, {(256, 1): 1, (384, 1): -1}),
            (32, {(0, 544): 0.5, (1, 544): 0.5}, {(544, 1): 1})],
    "D0a": [(96, {(0, 128): 1, (1, 128): -1}, {(128, 0): 1, (128, 1): 1}),
            (32, {(0, 224): 1, (1, 224): 1}, {(224, 0): 1, (224, 1): 1})],
    "D0b": [(96, {(0, 384): 1, (1, 384): -1}, {(384, 0): 1, (384, 1): -1}),
            (32, {(0, 480): 1, (1, 480): 1}, {(480, 0): 1, (480, 1): -1})],
    "D1a": [(96, {(1, 0): 1, (0, 0): -1}, {(0, 0): 1, (0, 1): 1}),
            (32, {(1, 96): 1, (0, 96): 1}, {(96, 0): 1, (96, 1): 1})],
    "D1b": [(96, {(0, 256): 1, (1, 256): -1}, {(256, 0): 1, (256, 1): -1}),
            (32, {(1, 352): -1, (0, 352): -1}, {(352, 0): 1, (352, 1): -1})],
}
FULL = tuple(n for n in PASSES if n[2:] not in ("a", "b"))
DOUBLE = ("K0", "K1", "D0", "D1")
TICKS = 60


def prepare_weights(wbuf, bbuf, wops, wk, bias_ref, wcp=(), wsplit=(), bcp=None):
    D, F = wbuf.shape
    H = F // 2
    Q = H // 2
    tiles = [None] * 5
    todo = list(zip(wcp, wsplit))
    for k0 in (512, 0, 128, 256, 384):
        for cp, (lo, n) in list(todo):
            if lo <= k0 < lo + n:
                cp.wait()
                todo.remove((cp, (lo, n)))
        wp = pltpu.bitcast(jnp.concatenate(_prune_rows(wbuf[k0:min(k0 + 128, D), :]), axis=0), BF16)
        if k0 == 512:
            if bcp is not None:
                bcp.wait()
            bias = jnp.broadcast_to(bbuf[...].reshape(1, F).astype(F32), (64, F)).astype(BF16)
            wp = jnp.concatenate([wp, bias], axis=0)
        tiles[k0 // 128] = wp.T
    tiles = [t.astype(F32) for t in tiles]
    lane = lax.broadcasted_iota(I32, (H, 128), 1)
    lane2 = lax.broadcasted_iota(I32, (F, 128), 1)
    bias_ref[...] = jnp.where(lane2 < 64, pltpu.roll(tiles[4], 64, 1), tiles[4])

    def operand(nm):
        pos, res = 0, None
        for h, a, _ in PASSES[nm]:
            v = None
            for (i, o), c in sorted(a.items(), key=lambda kv: -kv[1]):
                t = tiles[o // 128][i * H:(i + 1) * H]
                if v is None:
                    v, s = t, c
                else:
                    v = v + t if c == s else v - t
                off = o % 128
            if s != 1:
                v = v * s
            if off != pos:
                v = pltpu.roll(v, (pos - off) % 128, 1)
            res = v if res is None else jnp.where(lane < pos, res, v)
            pos += h
        return res

    for p, nm in enumerate(FULL):
        wops[p] = pltpu.bitcast(operand(nm).astype(BF16), I32)
    for j, nm in enumerate(DOUBLE):
        a, b = operand(nm + "a"), operand(nm + "b")
        a0, a1, b0, b1 = a[:Q], a[Q:], b[:Q], b[Q:]
        for i, v in enumerate((a0 + b1, a1 + b1, a0, b1, a0 + b0, a1 - a0, b0 - b1)):
            wk[7 * j + i] = pltpu.bitcast(v.astype(BF16), I32)


def pair(wops, wk, bias_ref, xload, ostore, tick, order="C"):
    H = bias_ref.shape[0] // 2

    def xparts(nm, u):
        parts = []
        for h, _, b in PASSES[nm]:
            items = list(b.items())
            if len(items) == 1:
                parts.append(xload(u, h, *items[0][0]))
            else:
                p, q = (xload(u, h, *k).astype(F32) for k, _ in items)
                parts.append(p + q if items[1][1] > 0 else p - q)
        return parts

    def dot(w, parts):
        x = jnp.concatenate([p.astype(BF16) for p in parts], axis=0)
        return jnp.dot(pltpu.bitcast(w, BF16), x, preferred_element_type=F32)

    def mm(nm, u):
        tick(2)
        if nm[0] == "R":
            (k0, j), = PASSES[nm][0][2]
            return dot(wops[FULL.index(nm)], [xload(u, 128, k0, j)])
        return dot(wops[FULL.index(nm)], xparts(nm, u))

    def strassen(nm):
        j = DOUBLE.index(nm)
        a, b = nm + "a", nm + "b"

        def m(i, p, sign=0, q=None):
            tick(1)
            parts = xparts(*p)
            if q is not None:
                parts = [x.astype(F32) + y.astype(F32) if sign > 0 else x.astype(F32) - y.astype(F32)
                         for x, y in zip(parts, xparts(*q))]
            return dot(wk[7 * j + i], parts)

        m2 = m(1, (a, 0))
        m4 = m(3, (b, 0), -1, (a, 0))
        m1 = m(0, (a, 0), 1, (b, 1))
        m7 = m(6, (b, 0), 1, (b, 1))
        c10 = m2 + m4; t00 = (m1 + m4) + m7; t11 = m1 - m2
        m5 = m(4, (b, 1))
        m3 = m(2, (a, 1), -1, (b, 1))
        m6 = m(5, (a, 0), 1, (a, 1))
        c00 = t00 - m5; c01 = m3 + m5; c11 = (m3 + m6) + t11
        return jnp.concatenate([c00, c10], axis=0), jnp.concatenate([c01, c11], axis=0)

    def rows(u):
        p0 = mm("R0p", u) + bias_ref[0:H, :]; n0 = mm("R0n", u)
        p1 = mm("R1p", u) + bias_ref[H:, :]; m1 = mm("R1m", u)
        return p0 - n0, p0 + n0, p1 + m1, p1 - m1

    def cols(u, k0, k1, d0, d1):
        gp = mm("Gp", u); gm = mm("Gm", u); m0 = mm("K0m", u); m1 = mm("K1m", u)
        return (((gp + gm) + m0) + (k0[u] + d0[u]), k1[u] + m1, k0[u] - m0,
                ((gp - gm) - m1) + (k1[u] + d1[u]))

    def emit(u, r, c):
        o = [x + y for x, y in zip(c, r)]
        ostore(u, jnp.concatenate(o[:2], axis=1).astype(BF16), jnp.concatenate(o[2:], axis=1).astype(BF16))

    if order == "B":
        s = [strassen(n) for n in DOUBLE]
        for u in range(2):
            c = cols(u, *s)
            emit(u, rows(u), c)
    elif order == "C":
        r = [rows(0), rows(1)]
        s = [strassen(n) for n in DOUBLE]
        for u in range(2):
            emit(u, r[u], cols(u, *s))
    elif order == "D":
        r0 = rows(0)
        s = [strassen(n) for n in DOUBLE]
        emit(0, r0, cols(0, *s))
        c = cols(1, *s)
        emit(1, rows(1), c)
    elif order == "E":
        r0 = rows(0)
        s = [strassen(n) for n in DOUBLE]
        r1 = rows(1)
        emit(0, r0, cols(0, *s))
        emit(1, r1, cols(1, *s))


PAIR = 512
G = 64


def _kernel(x_hbm, w_hbm, b_hbm, o_hbm, xbuf, obuf, wbuf, bbuf, wops, wk, bias_ref, isem, osem, wsem,
            *, pos, rlead, stop, mode, order, order0, csem, wcount, early, wsplit, wch, lch, early_last, el_at,
            lastprio, a1):
    D = w_hbm.shape[0]
    S = x_hbm.shape[2]
    NG = D // G
    NB = x_hbm.shape[0] // NG
    RX = xbuf.shape[0] // NG
    H = D // 2
    HALF = NB // 2
    npair = S // PAIR
    NP = 64
    assert len(pos) * npair == NP
    scope = jax.named_scope if "prof" in mode else (lambda n: contextlib.nullcontext())

    def xslot(t):
        return (t % RX if isinstance(t, int) else jnp.where(t >= RX, t - RX, t)) * NG

    def icopy(t, r, c, k):
        if not isinstance(r, int):
            r, c = pl.multiple_of(r, 8), pl.multiple_of(c, PAIR)
        idx = (pl.ds(r, 8), pl.ds(c, PAIR))
        return pltpu.make_async_copy(x_hbm.at[(pl.ds(t * NG, NG), *idx)], xbuf.at[(pl.ds(xslot(t), NG), *idx)],
                                     isem.at[k])

    first_b = [(0, 8 * r, c * PAIR, NB + csem[c]) for c in range(npair) for r in range(0 if c < 2 else 4, 8)]
    first_b += [(1, 8 * r, c * PAIR, 1) for r in range(5, 8) for c in range(npair)]
    first_a = [(0, 8 * r, c * PAIR, NB + csem[c]) for c in range(2, npair) for r in range(4)]
    first_a += [(1, 8 * r, c * PAIR, 1) for r in range(5) for c in range(npair)]
    piece = [(8 * r, c * PAIR) for r in range(8) for c in range(npair)]

    bcp = pltpu.make_async_copy(b_hbm, bbuf, wsem.at[0])
    wcp = [pltpu.make_async_copy(w_hbm.at[pl.ds(k0, n)], wbuf.at[pl.ds(k0, n)], wsem.at[1 + i])
           for i, (k0, n) in enumerate(wsplit)]
    bcp.start()
    for cp in wcp:
        cp.start()
    assert 16 <= rlead <= 40

    def pro(i, c):
        ch = jnp.where(i < 16, i >> 3, (i >> 2) - 2)
        r = jnp.where(i < 16, i & 7, (i & 3) + 4)
        k = NB + ch
        for c0 in range(npair):
            if csem[c0] != c0:
                k = jnp.where(ch == c0, NB + csem[c0], k)
        icopy(0, r * 8, ch * PAIR, k).start(priority=1)
        return c

    lax.fori_loop(0, rlead, pro, 0)
    with scope("prep"):
        prepare_weights(wbuf, bbuf, wops, wk, bias_ref, wcp, wsplit, bcp)

    def ocopy(rows, g0, r0, c0, nc):
        idx = (pl.ds(g0, NG), pl.ds(r0, 8), pl.ds(c0, nc))
        shape = (NB * D // rows, rows, S)
        return pltpu.make_async_copy(obuf.reshape(*shape).at[idx], o_hbm.reshape(*shape).at[idx], osem.at[0])

    def batch_wait(t):
        v = xbuf.at[pl.ds(xslot(t), NG)]
        pltpu.make_async_copy(v, v, isem.at[t]).wait()

    wdescs = [(r0, c0) for r0 in range(0, 2 * G, 8) for c0 in range(0, S, wch)]
    ldescs = [(r0, c0) for r0 in range(0, G, 8) for c0 in range(0, S, lch)]
    assert sum(wcount) == len(wdescs)

    def body(t, carry):
        state = {"tick": 0, "paced": 0, "w": 0}
        first = t == 0
        xs = xslot(t)
        row0 = pl.multiple_of(t * D, G)

        @pl.when(t > 0)
        def _():
            batch_wait(t)

        def pick(a, b):
            return [jnp.where(first, p, q) for p, q in zip(a, b)]

        def tick(n):
            q = state["tick"] % TICKS
            if n and q in (36, 52):
                write()
            for _ in range((pos.count(q) if n else pos.count(TICKS))):
                i = state["paced"]
                da = pick(first_a[i], (2 * t + 1, *piece[i], 2 * t + 1))
                cond = t < (HALF if i < NP - stop else HALF - 1)
                if i >= NP - a1:
                    cond = cond & (t > 0)

                @pl.when(cond)
                def _():
                    icopy(*da).start(priority=0)
                j = i + rlead
                if NP - a1 <= j < NP:
                    @pl.when(first)
                    def _():
                        icopy(*first_a[j]).start(priority=1)
                if j < NP:
                    db = pick(first_b[j], (2 * t, *piece[j], 2 * t))

                    @pl.when(t < HALF)
                    def _():
                        icopy(*db).start(priority=1)
                else:
                    @pl.when(t < HALF - 1)
                    def _():
                        icopy(2 * t + 2, *piece[j - NP], 2 * t + 2).start(priority=1)
                    if j - NP < stop:
                        @pl.when(t == HALF - 1)
                        def _():
                            icopy(NB - 1, *piece[j - stop], NB - 1).start(priority=1)
                state["paced"] += 1
            state["tick"] += n

        npt = 2 * npair + 1

        def write():
            if "rdonly" in mode:
                return
            i = state["w"]
            j = (i + early) % npt
            k = t - HALF + (i + early) // npt
            lo = sum(wcount[:j])
            for r0, c0 in wdescs[lo:lo + wcount[j]]:
                @pl.when((k >= 0) & (k < HALF - 1))
                def _():
                    ocopy(2 * G, k * NG, r0, c0, wch).start()
            if i + early < npt:
                n = -(-len(ldescs) // 8)
                for r0, c0 in ldescs[i * n:(i + 1) * n]:
                    @pl.when(t == NB - 1)
                    def _():
                        ocopy(G, (NB - 2) * NG, r0, c0, lch).start()
            if early_last and el_at <= i < npt - 1:
                ds = [d for d in ldescs if d[1] < early_last]
                n = -(-len(ds) // (npt - 1 - el_at))
                for r0, c0 in ds[(i - el_at) * n:(i - el_at + 1) * n]:
                    @pl.when(t == NB - 1)
                    def _():
                        ocopy(G, (NB - 1) * NG, r0, c0, lch).start()
            state["w"] += 1

        for p in range(npair):
            o = p * PAIR
            if csem[p] == p:
                @pl.when(first)
                def _():
                    v = xbuf.at[pl.ds(0, NG), :, pl.ds(o, PAIR * csem.count(p))]
                    pltpu.make_async_copy(v, v, isem.at[NB + p]).wait()

            def xload(u, h, k0, j):
                c = o + u * 256 + j * 128
                parts, k = [], k0
                while k < k0 + h:
                    g, r = divmod(k, G)
                    n = min(G - r, k0 + h - k)
                    parts.append(xbuf[xs + g, r:r + n, c:c + 128])
                    k += n
                return jnp.concatenate(parts, axis=0)

            def ostore(u, v0, v1):
                c = o + u * 256
                if len(obuf.shape) == 2:
                    obuf[pl.ds(row0, H), c:c + 256] = v0
                    obuf[pl.ds(row0 + H, H), c:c + 256] = v1
                else:
                    v = jnp.concatenate([v0, v1], axis=0)
                    for g in range(NG):
                        obuf[t * NG + g, :, c:c + 256] = v[g * G:(g + 1) * G]

            pair(wops, wk, bias_ref, xload, ostore, tick, order if p else order0)
            tick(0)
        write()
        return carry

    def sbody(t, c):
        with scope("iter"):
            return body(t, c)

    if "rdonly" in mode:
        lax.fori_loop(0, HALF, sbody, 0)
        with scope("rdwait"):
            for q in range(HALF, NB):
                batch_wait(q)
        cp = pltpu.make_async_copy(obuf.at[0, :16, :128], o_hbm.at[0, :16, :128], osem.at[0])
        cp.start()
        cp.wait()
        return
    lax.fori_loop(0, NB, sbody, 0)
    with scope("tail"):
        for r0, c0 in ldescs:
            if c0 >= early_last:
                ocopy(G, (NB - 1) * NG, r0, c0, lch).start(priority=lastprio)
        pltpu.make_async_copy(obuf, obuf, osem.at[0]).wait()


def make(RX=10, o3d=True, pad=0, flags=("XLA_TPU_RESCHEDULE_DMA_DONES",), **kw):
    cfg = dict(pos=(0, 8, 16, 24, 28, 36, 44, 52), rlead=32, stop=4, early_last=0, el_at=14,
               mode="", order="B", order0="D", csem=(0, 1, 2, 3, 4, 4, 6, 6),
               wcount=(8, 2, 6, 2, 6, 2, 6, 2, 6, 2, 6, 2, 6, 2, 6, 0, 0), early=1, wch=1024, lch=512,
               lastprio=0, a1=0,
               wsplit=((512, 64), (0, 128), (128, 128), (256, 128), (384, 128)))
    cfg.update(kw)

    def fn(x, w, b):
        B, S, D = x.shape
        F = w.shape[1]
        xt = jnp.transpose(x, (0, 2, 1)).reshape(B * D // G, G, S)
        oshape = (B * F // G, G, S) if o3d else (B * F, S)
        out = pl.pallas_call(
            functools.partial(_kernel, **cfg),
            in_specs=[pl.BlockSpec(memory_space=pl.ANY)] * 3,
            out_specs=pl.BlockSpec(memory_space=pl.ANY),
            out_shape=jax.ShapeDtypeStruct(oshape, x.dtype),
            scratch_shapes=[
                pltpu.VMEM((RX * D // G, G, S), x.dtype),
                pltpu.VMEM(oshape, x.dtype),
                pltpu.VMEM((D, F), w.dtype),
                pltpu.VMEM((F,), b.dtype),
                pltpu.VMEM((len(FULL), F // 4, 128), I32),
                pltpu.VMEM((28, F // 8, 128), I32),
                pltpu.VMEM((F, 128), F32),
                pltpu.SemaphoreType.DMA((B + S // PAIR,)),
                pltpu.SemaphoreType.DMA((1,)),
                pltpu.SemaphoreType.DMA((len(cfg["wsplit"]) + 1,)),
            ],
            compiler_params=pltpu.CompilerParams(
                vmem_limit_bytes=127 * 1024 * 1024,
                flags={k: True for k in flags} or None,
                disable_bounds_checks=True,
                disable_semaphore_checks=True,
            ),
            name="k5",
        )(xt, w, b)
        return jnp.transpose(out.reshape(B, F, S), (0, 2, 1))
    return fn


@jax.jit
def pallas_standalone__structured_sparse_n_m__ragged_kernel(
    x: jax.Array,
    w: jax.Array,
    b: jax.Array,
):
    return make(stop=6)(x, w, b)
```

```python
import jax
import jax.numpy as jnp
from jax import lax
import jax.experimental.pallas as pl
import jax.experimental.pallas.tpu as pltpu

F32, BF16, I32 = jnp.float32, jnp.bfloat16, jnp.int32

_PASSES = {
    "Gp": [(96, {(0, 0): 1, (1, 128): 1}, {(0, 0): 1, (128, 1): 1}),
           (32, {(0, 352): 1, (1, 480): -1}, {(352, 0): 1, (480, 1): -1})],
    "Gm": [(96, {(0, 256): 1, (1, 384): 1}, {(256, 0): 1, (384, 1): -1}),
           (32, {(0, 96): 1, (1, 224): -1}, {(96, 0): 1, (224, 1): 1})],
    "R0p": [(128, {(0, 256): 1, (0, 384): 1}, {(384, 1): 1})],
    "R0m": [(128, {(0, 0): 1, (0, 128): 1}, {(128, 1): 1})],
    "R1p": [(128, {(1, 256): 1, (1, 384): 1}, {(256, 0): 1})],
    "R1m": [(128, {(1, 0): 1, (1, 128): 1}, {(0, 0): 1})],
    "C0m": [(64, {(0, 512): 0.5, (1, 512): -0.5}, {(512, 0): 1}),
            (32, {(1, 224): 1}, {(96, 0): 1, (224, 0): -1}),
            (32, {(1, 480): 1}, {(352, 0): 1, (480, 0): -1})],
    "C1m": [(64, {(0, 512): 0.5, (1, 512): -0.5}, {(512, 1): 1}),
            (32, {(0, 96): 1}, {(96, 1): 1, (224, 1): -1}),
            (32, {(0, 352): 1}, {(352, 1): 1, (480, 1): -1})],
    "C0a": [(96, {(1, 128): 1}, {(128, 0): 1, (0, 0): -1}),
            (32, {(0, 512): 0.5, (1, 512): 0.5}, {(512, 0): 1})],
    "C0b": [(96, {(1, 384): 1}, {(384, 0): 1, (256, 0): -1}),
            (32, {(0, 544): 0.5, (1, 544): 0.5}, {(544, 0): 1})],
    "C1a": [(96, {(0, 0): 1}, {(0, 1): 1, (128, 1): -1}),
            (32, {(0, 512): 0.5, (1, 512): 0.5}, {(512, 1): 1})],
    "C1b": [(96, {(0, 256): 1}, {(256, 1): 1, (384, 1): -1}),
            (32, {(0, 544): 0.5, (1, 544): 0.5}, {(544, 1): 1})],
    "D0a": [(96, {(0, 128): 1, (1, 128): -1}, {(128, 0): 1, (128, 1): 1}),
            (32, {(0, 224): 1, (1, 224): 1}, {(224, 0): 1, (224, 1): 1})],
    "D0b": [(96, {(0, 384): 1, (1, 384): -1}, {(384, 0): 1, (384, 1): -1}),
            (32, {(0, 480): 1, (1, 480): 1}, {(480, 0): 1, (480, 1): -1})],
    "D1a": [(96, {(1, 0): 1, (0, 0): -1}, {(0, 0): 1, (0, 1): 1}),
            (32, {(1, 96): 1, (0, 96): 1}, {(96, 0): 1, (96, 1): 1})],
    "D1b": [(96, {(0, 256): 1, (1, 256): -1}, {(256, 0): 1, (256, 1): -1}),
            (32, {(1, 352): -1, (0, 352): -1}, {(352, 0): 1, (352, 1): -1})],
}
_SINGLE = ("Gp", "Gm", "R0p", "R0m", "R1p", "R1m", "C0m", "C1m")
_DOUBLE = ("C0", "C1", "D0", "D1")

_XG = 64
_OG = 128
_CHUNK = 512
_OCHUNK = 1024
_XRING = 5
_W_ROWS = ((512, 64), (0, 128), (128, 128), (256, 128), (384, 128))
_STEPS = ((0, 0), (0, 1), (1, 0), (1, 1), (0, 2), (1, 2), (0, 3), (1, 3))
_READ_AT = (0, 8, 16, 24, 28, 36, 44, 52)
_WRITE_AT = {36: 2, 52: 6}
_LATE = 5


def _prune(w):
    words = pltpu.bitcast(w, I32)
    mate = lax.broadcasted_iota(I32, (8, w.shape[1]), 0) ^ 1
    parts = []
    for i in range(0, words.shape[0], 8):
        u = words[i:i + 8]
        lo = pltpu.bitcast((u << 16) & 0x7FFFFFFF, F32)
        hi = pltpu.bitcast(u & 0x7FFF0000, F32)
        big, small = jnp.maximum(lo, hi), jnp.minimum(lo, hi)
        nbig = jnp.take_along_axis(big, mate, axis=0, mode="promise_in_bounds")
        nsmall = jnp.take_along_axis(small, mate, axis=0, mode="promise_in_bounds")
        thr = jnp.maximum(jnp.minimum(big, nbig), jnp.maximum(small, nsmall))
        parts.append(u & (jnp.where(lo < thr, 0, 0xFFFF) | jnp.where(hi < thr, 0, -65536)))
    return pltpu.bitcast(jnp.concatenate(parts, axis=0), BF16)


def _prepare_weights(w_copies, b_copy, wbuf, bbuf, w1_ref, w2_ref, bias_ref):
    F = wbuf.shape[1]
    H = F // 2
    tiles = {}
    for cp, (k0, n) in zip(w_copies, _W_ROWS):
        cp.wait()
        wp = _prune(wbuf[k0:k0 + n, :])
        if n < 128:
            b_copy.wait()
            bias = jnp.broadcast_to(bbuf[...].reshape(1, F).astype(F32), (128 - n, F))
            wp = jnp.concatenate([wp, bias.astype(BF16)], axis=0)
        tiles[k0] = wp.T
    tiles = {k0: t.astype(F32) for k0, t in tiles.items()}
    low = lax.broadcasted_iota(I32, (F, 128), 1) < 64
    bias_ref[...] = jnp.where(low, pltpu.roll(tiles[512], 64, 1), tiles[512])
    lane = lax.broadcasted_iota(I32, (H, 128), 1)

    def operand(name):
        pos, res = 0, None
        for depth, coefs, _ in _PASSES[name]:
            ((i, k), scale), *rest = coefs.items()
            v = tiles[k - k % 128][i * H:(i + 1) * H]
            for (i2, k2), c in rest:
                t = tiles[k2 - k2 % 128][i2 * H:(i2 + 1) * H]
                v = v + t if c == scale else v - t
            if scale != 1:
                v = v * scale
            if k % 128 != pos:
                v = pltpu.roll(v, (pos - k) % 128, 1)
            res = v if res is None else jnp.where(lane < pos, res, v)
            pos += depth
        return res

    for p, name in enumerate(_SINGLE):
        w1_ref[p] = pltpu.bitcast(operand(name).astype(BF16), I32)
    for p, name in enumerate(_DOUBLE):
        a, b = operand(name + "a"), operand(name + "b")
        a0, a1, b0, b1 = a[:H // 2], a[H // 2:], b[:H // 2], b[H // 2:]
        for i, v in enumerate((a1 + b1, b1, a0 + b1, b0 - b1, a0 + b0, a0, a1 - a0)):
            w2_ref[7 * p + i] = pltpu.bitcast(v.astype(BF16), I32)


def _tokens512(w1_ref, w2_ref, bias_ref, load_x, store_out, tick, plain_first):
    H = bias_ref.shape[0] // 2

    def x_operand(name, u):
        parts = []
        for depth, _, signs in _PASSES[name]:
            (first, _), *rest = signs.items()
            v = load_x(u, depth, *first)
            for other, sign in rest:
                v, q = v.astype(F32), load_x(u, depth, *other).astype(F32)
                v = v + q if sign > 0 else v - q
            parts.append(v)
        return parts

    def dot(w, parts):
        x = jnp.concatenate([p.astype(BF16) for p in parts], axis=0)
        return jnp.dot(pltpu.bitcast(w, BF16), x, preferred_element_type=F32)

    def single(name, u):
        tick(2)
        return dot(w1_ref[_SINGLE.index(name)], x_operand(name, u))

    def double(name):
        u, v = (0, 1) if name[0] == "C" else (1, 0)
        xa, xb = name + "a", name + "b"

        def m(i, p, sign=0, q=None):
            tick(1)
            parts = x_operand(*p)
            if q is not None:
                pairs = [(s.astype(F32), t.astype(F32)) for s, t in zip(parts, x_operand(*q))]
                parts = [s + t if sign > 0 else s - t for s, t in pairs]
            return dot(w2_ref[7 * _DOUBLE.index(name) + i], parts)

        m2 = m(0, (xa, u))
        m4 = m(1, (xb, u), -1, (xa, u))
        m1 = m(2, (xa, u), 1, (xb, v))
        m7 = m(3, (xb, u), 1, (xb, v))
        low_u, top_u, low_v = m2 + m4, (m1 + m4) + m7, m1 - m2
        m5 = m(4, (xb, v))
        m3 = m(5, (xa, v), -1, (xb, v))
        m6 = m(6, (xa, u), 1, (xa, v))
        return {u: jnp.concatenate([top_u - m5, low_u], axis=0),
                v: jnp.concatenate([m3 + m5, (m3 + m6) + low_v], axis=0)}

    def rows(u):
        p0, m0 = single("R0p", u) + bias_ref[0:H, :], single("R0m", u)
        p1, m1 = single("R1p", u) + bias_ref[H:, :], single("R1m", u)
        return p0 - m0, p0 + m0, p1 + m1, p1 - m1

    def rest(u, c0, c1, d0, d1):
        gp, gm, m0, m1 = (single(name, u) for name in ("Gp", "Gm", "C0m", "C1m"))
        return (((gp + gm) + m0) + (c0[u] + d0[u]), c1[u] + m1,
                c0[u] - m0, ((gp - gm) - m1) + (c1[u] + d1[u]))

    done = {0: rows(0)} if plain_first else {}
    doubles = [double(name) for name in _DOUBLE]
    for u in range(2):
        c = rest(u, *doubles)
        c = [s + t for s, t in zip(c, done[u] if u in done else rows(u))]
        halves = [jnp.concatenate(c[i:i + 2], axis=1).astype(BF16) for i in (0, 2)]
        store_out(u, jnp.concatenate(halves, axis=0))


def _kernel(x_hbm, w_hbm, b_hbm, o_hbm, xbuf, obuf, wbuf, bbuf, w1_ref, w2_ref, bias_ref,
            xsem, osem, wsem):
    D, F = w_hbm.shape
    S = x_hbm.shape[2]
    XN, ON = D // _XG, 2 * F // _OG
    B = x_hbm.shape[0] // XN
    half = S // 2
    tiles = _XG // 8
    chunks = half // _CHUNK
    pieces = [(8 * r, _CHUNK * c) for r in range(tiles) for c in range(2 * chunks)]
    early = ([(8 * r, _CHUNK * c) for c in range(chunks) for r in range(tiles)]
             + [p for p in pieces if p[1] >= half])
    NP = len(pieces)

    def select(pred, p, q, col_align):
        row, col = (jnp.where(pred, a, b) for a, b in zip(p, q))
        return pl.multiple_of(row, 8), pl.multiple_of(col, col_align)

    def ring(k):
        return jnp.where(k >= _XRING, k - _XRING, k)

    def x_copy(k, i, row, col, sem):
        window = (pl.ds(row, 8), pl.ds(col, _CHUNK))
        return pltpu.make_async_copy(x_hbm.at[(pl.ds((2 * k + i) * XN, XN), *window)],
                                     xbuf.at[(pl.ds((2 * ring(k) + i) * XN, XN), *window)],
                                     xsem.at[sem])

    def x_wait(g0, col, n, sem):
        dst = xbuf.at[pl.ds(g0, XN), :, pl.ds(col, n)]
        pltpu.make_async_copy(dst, dst, xsem.at[sem]).wait()

    def out_copy(k, row, col):
        window = (pl.ds(k * ON, ON), pl.ds(row, 8), pl.ds(col, _OCHUNK))
        return pltpu.make_async_copy(obuf.at[window], o_hbm.at[window], osem.at[0])

    out_pieces = [(r, c) for r in range(0, _OG, 8) for c in range(0, S, _OCHUNK)]
    out_halves = [[p for p in out_pieces if p[1] // half == h] for h in range(2)]

    b_copy = pltpu.make_async_copy(b_hbm, bbuf, wsem.at[0])
    w_copies = [pltpu.make_async_copy(w_hbm.at[pl.ds(k0, n)], wbuf.at[pl.ds(k0, n)], wsem.at[1 + i])
                for i, (k0, n) in enumerate(_W_ROWS)]
    b_copy.start()
    for cp in w_copies:
        cp.start()

    def first_reads(c, carry):
        for r in range(tiles):
            x_copy(0, 0, 8 * r, pl.multiple_of(c * _CHUNK, _CHUNK), 2 * B + c).start(priority=1)
        return carry

    lax.fori_loop(0, chunks, first_reads, 0)
    _prepare_weights(w_copies, b_copy, wbuf, bbuf, w1_ref, w2_ref, bias_ref)

    def step(t, carry):
        k, h = t >> 1, t & 1
        first = t == 0
        xg = 2 * XN * ring(k)
        col = pl.multiple_of(h * half, half)
        xs = xbuf.at[pl.ds(xg, 2 * XN), :, pl.ds(col, half)]
        os_ = obuf.at[pl.ds(k * ON, ON), :, pl.ds(col, half)]
        count = {"ticks": 0, "reads": 0, "writes": 0}

        def read():
            i = count["reads"]
            count["reads"] += 1
            ahead, j = divmod(i + NP // 2, NP)

            @pl.when(t < B // 2 - int(i >= NP - _LATE))
            def _():
                sem = 2 * B + chunks + i // tiles if early[i][1] < half else 3
                sem = jnp.where(first, sem, 4 * t + 2 + pieces[i][1] // half)
                x_copy(t, 1, *select(first, early[i], pieces[i], _CHUNK), sem).start(priority=0)

            @pl.when(t < B // 2 - ahead)
            def _():
                sem = 4 * (t + ahead) + pieces[j][1] // half
                if ahead:
                    x_copy(t + 1, 0, *pieces[j], sem).start(priority=1)
                else:
                    x_copy(t, 0, *select(first, early[j], pieces[j], _CHUNK),
                           jnp.where(first, 1, sem)).start(priority=1)

            if ahead and j < _LATE:
                @pl.when(t == B // 2 - 1)
                def _():
                    row, c = pieces[NP - _LATE + j]
                    x_copy(t, 1, row, c, 4 * t + 2 + c // half).start(priority=1)

        def write(n, pair):
            for _ in range(n):
                i = count["writes"] % len(out_pieces)
                count["writes"] += 1
                last = i < len(out_halves[0])

                @pl.when((pair >= 0) & (pair < B // 2 - 1 + last))
                def _():
                    piece = out_pieces[i]
                    if last:
                        piece = select(pair == B // 2 - 1, out_halves[0][i], piece, _OCHUNK)
                    out_copy(pair, *piece).start()

        def tick(n):
            pos = count["ticks"] % 60
            count["ticks"] += n
            write(_WRITE_AT.get(pos, 0) * (count["writes"] < len(out_pieces)), t - B // 2)
            if pos in _READ_AT:
                read()

        lead = sum(_WRITE_AT.values())
        assert lead * len(_STEPS) == len(out_pieces) and len(_READ_AT) * len(_STEPS) == NP
        count["writes"] = lead
        for p, (i, c) in enumerate(_STEPS):
            @pl.when(first)
            def _():
                x_wait(i * XN, c * _CHUNK, _CHUNK, 2 * B + i * chunks + c)

            if c == 0:
                @pl.when(t > 0)
                def _():
                    x_wait(xg + i * XN, col, half, 4 * k + 2 * i + h)

            def load_x(u, n, k0, j):
                window = pl.ds(c * _CHUNK + 256 * u + 128 * j, 128)
                cuts = sorted({k0, k0 + n} | set(range(-(-k0 // _XG) * _XG, k0 + n, _XG)))
                return jnp.concatenate(
                    [xs[i * XN + lo // _XG, pl.ds(lo % _XG, hi - lo), window]
                     for lo, hi in zip(cuts, cuts[1:])], axis=0)

            def store_out(u, v):
                window = pl.ds(c * _CHUNK + 256 * u, 256)
                cuts = sorted({i * F, i * F + F} | set(range(-(-i * F // _OG) * _OG, i * F + F, _OG)))
                for lo, hi in zip(cuts, cuts[1:]):
                    os_[lo // _OG, pl.ds(lo % _OG, hi - lo), window] = v[lo - i * F:hi - i * F]

            _tokens512(w1_ref, w2_ref, bias_ref, load_x, store_out, tick, plain_first=p == 0)
        write(lead, t + 1 - B // 2)
        return carry

    lax.fori_loop(0, B, step, 0)
    for piece in out_halves[1]:
        out_copy(B // 2 - 1, *piece).start()
    pltpu.make_async_copy(obuf, obuf, osem.at[0]).wait()


@jax.jit
def pallas_standalone__structured_sparse_n_m__ragged_kernel(
    x: jax.Array,
    w: jax.Array,
    b: jax.Array,
):
    B, S, D = x.shape
    F = w.shape[1]
    xt = jnp.transpose(x, (0, 2, 1)).reshape(B * D // _XG, _XG, S)
    out = pl.pallas_call(
        _kernel,
        in_specs=[pl.BlockSpec(memory_space=pl.ANY)] * 3,
        out_specs=pl.BlockSpec(memory_space=pl.ANY),
        out_shape=jax.ShapeDtypeStruct((B * F // _OG, _OG, S), x.dtype),
        scratch_shapes=[
            pltpu.VMEM((2 * _XRING * D // _XG, _XG, S), x.dtype),
            pltpu.VMEM((B * F // _OG, _OG, S), x.dtype),
            pltpu.VMEM((D, F), w.dtype),
            pltpu.VMEM((F,), b.dtype),
            pltpu.VMEM((len(_SINGLE), F // 4, 128), I32),
            pltpu.VMEM((7 * len(_DOUBLE), F // 8, 128), I32),
            pltpu.VMEM((F, 128), F32),
            pltpu.SemaphoreType.DMA((2 * B + S // _CHUNK,)),
            pltpu.SemaphoreType.DMA((1,)),
            pltpu.SemaphoreType.DMA((1 + len(_W_ROWS),)),
        ],
        compiler_params=pltpu.CompilerParams(
            vmem_limit_bytes=124 * 1024 * 1024,
            flags={"XLA_TPU_RESCHEDULE_DMA_DONES": True},
            disable_bounds_checks=True,
            disable_semaphore_checks=True,
        ),
    )(xt, w, b)
    return jnp.transpose(out.reshape(B, F, S), (0, 2, 1))
```

```python
import jax
import jax.numpy as jnp
from jax import lax
import jax.experimental.pallas as pl
import jax.experimental.pallas.tpu as pltpu

F32, BF16, I32 = jnp.float32, jnp.bfloat16, jnp.int32

_PASSES = {
    "Gp": [(96, {(0, 0): 1, (1, 128): 1}, {(0, 0): 1, (128, 1): 1}),
           (32, {(0, 352): 1, (1, 480): -1}, {(352, 0): 1, (480, 1): -1})],
    "Gm": [(96, {(0, 256): 1, (1, 384): 1}, {(256, 0): 1, (384, 1): -1}),
           (32, {(0, 96): 1, (1, 224): -1}, {(96, 0): 1, (224, 1): 1})],
    "R0p": [(128, {(0, 256): 1, (0, 384): 1}, {(384, 1): 1})],
    "R0m": [(128, {(0, 0): 1, (0, 128): 1}, {(128, 1): 1})],
    "R1p": [(128, {(1, 256): 1, (1, 384): 1}, {(256, 0): 1})],
    "R1m": [(128, {(1, 0): 1, (1, 128): 1}, {(0, 0): 1})],
    "C0m": [(64, {(0, 512): 0.5, (1, 512): -0.5}, {(512, 0): 1}),
            (32, {(1, 224): 1}, {(96, 0): 1, (224, 0): -1}),
            (32, {(1, 480): 1}, {(352, 0): 1, (480, 0): -1})],
    "C1m": [(64, {(0, 512): 0.5, (1, 512): -0.5}, {(512, 1): 1}),
            (32, {(0, 96): 1}, {(96, 1): 1, (224, 1): -1}),
            (32, {(0, 352): 1}, {(352, 1): 1, (480, 1): -1})],
    "C0a": [(96, {(1, 128): 1}, {(128, 0): 1, (0, 0): -1}),
            (32, {(0, 512): 0.5, (1, 512): 0.5}, {(512, 0): 1})],
    "C0b": [(96, {(1, 384): 1}, {(384, 0): 1, (256, 0): -1}),
            (32, {(0, 544): 0.5, (1, 544): 0.5}, {(544, 0): 1})],
    "C1a": [(96, {(0, 0): 1}, {(0, 1): 1, (128, 1): -1}),
            (32, {(0, 512): 0.5, (1, 512): 0.5}, {(512, 1): 1})],
    "C1b": [(96, {(0, 256): 1}, {(256, 1): 1, (384, 1): -1}),
            (32, {(0, 544): 0.5, (1, 544): 0.5}, {(544, 1): 1})],
    "D0a": [(96, {(0, 128): 1, (1, 128): -1}, {(128, 0): 1, (128, 1): 1}),
            (32, {(0, 224): 1, (1, 224): 1}, {(224, 0): 1, (224, 1): 1})],
    "D0b": [(96, {(0, 384): 1, (1, 384): -1}, {(384, 0): 1, (384, 1): -1}),
            (32, {(0, 480): 1, (1, 480): 1}, {(480, 0): 1, (480, 1): -1})],
    "D1a": [(96, {(1, 0): 1, (0, 0): -1}, {(0, 0): 1, (0, 1): 1}),
            (32, {(1, 96): 1, (0, 96): 1}, {(96, 0): 1, (96, 1): 1})],
    "D1b": [(96, {(0, 256): 1, (1, 256): -1}, {(256, 0): 1, (256, 1): -1}),
            (32, {(1, 352): -1, (0, 352): -1}, {(352, 0): 1, (352, 1): -1})],
}
_SINGLE = ("Gp", "Gm", "R0p", "R0m", "R1p", "R1m", "C0m", "C1m")
_DOUBLE = ("C0", "C1", "D0", "D1")

_XG = 64
_OG = 128
_CHUNK = 512
_OCHUNK = 1024
_XRING = 5
_W_ROWS = ((512, 64), (0, 128), (128, 128), (256, 128), (384, 128))
_STEPS = ((0, 0), (0, 1), (1, 0), (1, 1), (0, 2), (1, 2), (0, 3), (1, 3))
_READ_AT = (0, 8, 16, 24, 28, 36, 44, 52)
_WRITE_AT = {36: 2, 52: 6}
_LATE = 5


def _prune(w):
    words = pltpu.bitcast(w, I32)
    mate = lax.broadcasted_iota(I32, (8, w.shape[1]), 0) ^ 1
    parts = []
    for i in range(0, words.shape[0], 8):
        u = words[i:i + 8]
        lo = pltpu.bitcast((u << 16) & 0x7FFFFFFF, F32)
        hi = pltpu.bitcast(u & 0x7FFF0000, F32)
        big, small = jnp.maximum(lo, hi), jnp.minimum(lo, hi)
        nbig = jnp.take_along_axis(big, mate, axis=0, mode="promise_in_bounds")
        nsmall = jnp.take_along_axis(small, mate, axis=0, mode="promise_in_bounds")
        thr = jnp.maximum(jnp.minimum(big, nbig), jnp.maximum(small, nsmall))
        parts.append(u & (jnp.where(lo < thr, 0, 0xFFFF) | jnp.where(hi < thr, 0, -65536)))
    return pltpu.bitcast(jnp.concatenate(parts, axis=0), BF16)


def _prepare_weights(w_copies, b_copy, wbuf, bbuf, w1_ref, w2_ref, bias_ref):
    F = wbuf.shape[1]
    H = F // 2
    tiles = {}
    for cp, (k0, n) in zip(w_copies, _W_ROWS):
        cp.wait()
        wp = _prune(wbuf[k0:k0 + n, :])
        if n < 128:
            b_copy.wait()
            bias = jnp.broadcast_to(bbuf[...].reshape(1, F).astype(F32), (128 - n, F))
            wp = jnp.concatenate([wp, bias.astype(BF16)], axis=0)
        tiles[k0] = wp.T
    tiles = {k0: t.astype(F32) for k0, t in tiles.items()}
    low = lax.broadcasted_iota(I32, (F, 128), 1) < 64
    bias_ref[...] = jnp.where(low, pltpu.roll(tiles[512], 64, 1), tiles[512])
    lane = lax.broadcasted_iota(I32, (H, 128), 1)

    def operand(name):
        pos, res = 0, None
        for depth, coefs, _ in _PASSES[name]:
            ((i, k), scale), *rest = coefs.items()
            v = tiles[k - k % 128][i * H:(i + 1) * H]
            for (i2, k2), c in rest:
                t = tiles[k2 - k2 % 128][i2 * H:(i2 + 1) * H]
                v = v + t if c == scale else v - t
            if scale != 1:
                v = v * scale
            if k % 128 != pos:
                v = pltpu.roll(v, (pos - k) % 128, 1)
            res = v if res is None else jnp.where(lane < pos, res, v)
            pos += depth
        return res

    for p, name in enumerate(_SINGLE):
        w1_ref[p] = pltpu.bitcast(operand(name).astype(BF16), I32)
    for p, name in enumerate(_DOUBLE):
        a, b = operand(name + "a"), operand(name + "b")
        a0, a1, b0, b1 = a[:H // 2], a[H // 2:], b[:H // 2], b[H // 2:]
        for i, v in enumerate((a1 + b1, b1, a0 + b1, b0 - b1, a0 + b0, a0, a0 - a1)):
            w2_ref[7 * p + i] = pltpu.bitcast(v.astype(BF16), I32)


def _tokens512(w1_ref, w2_ref, bias_ref, load_x, store_out, tick, plain_first):
    H = bias_ref.shape[0] // 2

    def x_operand(name, u):
        parts = []
        for depth, _, signs in _PASSES[name]:
            (first, _), *rest = signs.items()
            v = load_x(u, depth, *first)
            for other, sign in rest:
                v, q = v.astype(F32), load_x(u, depth, *other).astype(F32)
                v = v + q if sign > 0 else v - q
            parts.append(v)
        return parts

    def dot(w, parts):
        x = jnp.concatenate([p.astype(BF16) for p in parts], axis=0)
        return jnp.dot(pltpu.bitcast(w, BF16), x, preferred_element_type=F32)

    def single(name, u):
        tick(2)
        return dot(w1_ref[_SINGLE.index(name)], x_operand(name, u))

    def double(name):
        u, v = (0, 1) if name[0] == "C" else (1, 0)
        xa, xb = name + "a", name + "b"

        def m(i, p, q=None):
            tick(1)
            parts = x_operand(*p)
            if q is not None:
                parts = [s.astype(F32) - t.astype(F32) for s, t in zip(parts, x_operand(*q))]
            return dot(w2_ref[7 * _DOUBLE.index(name) + i], parts)

        m2, m4 = m(0, (xa, u)), m(1, (xb, u), (xa, u))
        m1, m7 = m(2, (xa, u), (xb, v)), m(3, (xb, u), (xb, v))
        low_u, top_u, low_v = m2 + m4, (m1 + m4) + m7, m2 - m1
        m5, m3, m6 = m(4, (xb, v)), m(5, (xa, v), (xb, v)), m(6, (xa, u), (xa, v))
        return {u: jnp.concatenate([top_u + m5, low_u], axis=0),
                v: jnp.concatenate([m3 + m5, (m3 + m6) + low_v], axis=0)}

    def rows(u):
        p0, m0 = single("R0p", u) + bias_ref[0:H, :], single("R0m", u)
        p1, m1 = single("R1p", u) + bias_ref[H:, :], single("R1m", u)
        return p0 - m0, p0 + m0, p1 + m1, p1 - m1

    def rest(u, c0, c1, d0, d1):
        gp, gm, m0, m1 = (single(name, u) for name in ("Gp", "Gm", "C0m", "C1m"))
        return (((gp + gm) + m0) + (c0[u] + d0[u]), c1[u] + m1,
                c0[u] - m0, ((gp - gm) - m1) + (c1[u] + d1[u]))

    done = {0: rows(0)} if plain_first else {}
    doubles = [double(name) for name in _DOUBLE]
    for u in range(2):
        c = rest(u, *doubles)
        c = [s + t for s, t in zip(c, done[u] if u in done else rows(u))]
        halves = [jnp.concatenate(c[i:i + 2], axis=1).astype(BF16) for i in (0, 2)]
        store_out(u, jnp.concatenate(halves, axis=0))


def _kernel(x_hbm, w_hbm, b_hbm, o_hbm, xbuf, obuf, wbuf, bbuf, w1_ref, w2_ref, bias_ref,
            xsem, osem, wsem):
    D, F = w_hbm.shape
    S = x_hbm.shape[2]
    XN, ON = D // _XG, 2 * F // _OG
    B = x_hbm.shape[0] // XN
    half = S // 2
    tiles = _XG // 8
    chunks = half // _CHUNK
    pieces = [(8 * r, _CHUNK * c) for r in range(tiles) for c in range(2 * chunks)]
    early = ([(8 * r, _CHUNK * c) for c in range(chunks) for r in range(tiles)]
             + [p for p in pieces if p[1] >= half])
    NP = len(pieces)

    def select(pred, p, q, col_align):
        row, col = (jnp.where(pred, a, b) for a, b in zip(p, q))
        return pl.multiple_of(row, 8), pl.multiple_of(col, col_align)

    def ring(k):
        return jnp.where(k >= _XRING, k - _XRING, k)

    def x_copy(k, i, row, col, sem):
        window = (pl.ds(row, 8), pl.ds(col, _CHUNK))
        return pltpu.make_async_copy(x_hbm.at[(pl.ds((2 * k + i) * XN, XN), *window)],
                                     xbuf.at[(pl.ds((2 * ring(k) + i) * XN, XN), *window)],
                                     xsem.at[sem])

    def x_wait(g0, col, n, sem):
        dst = xbuf.at[pl.ds(g0, XN), :, pl.ds(col, n)]
        pltpu.make_async_copy(dst, dst, xsem.at[sem]).wait()

    def out_copy(k, row, col):
        window = (pl.ds(k * ON, ON), pl.ds(row, 8), pl.ds(col, _OCHUNK))
        return pltpu.make_async_copy(obuf.at[window], o_hbm.at[window], osem.at[0])

    out_pieces = [(r, c) for r in range(0, _OG, 8) for c in range(0, S, _OCHUNK)]
    out_halves = [[p for p in out_pieces if p[1] // half == h] for h in range(2)]

    b_copy = pltpu.make_async_copy(b_hbm, bbuf, wsem.at[0])
    w_copies = [pltpu.make_async_copy(w_hbm.at[pl.ds(k0, n)], wbuf.at[pl.ds(k0, n)], wsem.at[1 + i])
                for i, (k0, n) in enumerate(_W_ROWS)]
    b_copy.start()
    for cp in w_copies:
        cp.start()

    def first_reads(c, carry):
        for r in range(tiles):
            x_copy(0, 0, 8 * r, pl.multiple_of(c * _CHUNK, _CHUNK), 2 * B + c).start(priority=1)
        return carry

    lax.fori_loop(0, chunks, first_reads, 0)
    _prepare_weights(w_copies, b_copy, wbuf, bbuf, w1_ref, w2_ref, bias_ref)

    def step(t, carry):
        k, h = t >> 1, t & 1
        first = t == 0
        xg = 2 * XN * ring(k)
        col = pl.multiple_of(h * half, half)
        xs = xbuf.at[pl.ds(xg, 2 * XN), :, pl.ds(col, half)]
        os_ = obuf.at[pl.ds(k * ON, ON), :, pl.ds(col, half)]
        count = {"ticks": 0, "reads": 0, "writes": 0}

        def read():
            i = count["reads"]
            count["reads"] += 1
            ahead, j = divmod(i + NP // 2, NP)

            @pl.when(t < B // 2 - int(i >= NP - _LATE))
            def _():
                sem = 2 * B + chunks + i // tiles if early[i][1] < half else 3
                sem = jnp.where(first, sem, 4 * t + 2 + pieces[i][1] // half)
                x_copy(t, 1, *select(first, early[i], pieces[i], _CHUNK), sem).start(priority=0)

            @pl.when(t < B // 2 - ahead)
            def _():
                sem = 4 * (t + ahead) + pieces[j][1] // half
                if ahead:
                    x_copy(t + 1, 0, *pieces[j], sem).start(priority=1)
                else:
                    x_copy(t, 0, *select(first, early[j], pieces[j], _CHUNK),
                           jnp.where(first, 1, sem)).start(priority=1)

            if ahead and j < _LATE:
                @pl.when(t == B // 2 - 1)
                def _():
                    row, c = pieces[NP - _LATE + j]
                    x_copy(t, 1, row, c, 4 * t + 2 + c // half).start(priority=1)

        def write(n, pair):
            for _ in range(n):
                i = count["writes"] % len(out_pieces)
                count["writes"] += 1
                last = i < len(out_halves[0])

                @pl.when((pair >= 0) & (pair < B // 2 - 1 + last))
                def _():
                    piece = out_pieces[i]
                    if last:
                        piece = select(pair == B // 2 - 1, out_halves[0][i], piece, _OCHUNK)
                    out_copy(pair, *piece).start()

        def tick(n):
            pos = count["ticks"] % 60
            count["ticks"] += n
            write(_WRITE_AT.get(pos, 0) * (count["writes"] < len(out_pieces)), t - B // 2)
            if pos in _READ_AT:
                read()

        lead = sum(_WRITE_AT.values())
        assert lead * len(_STEPS) == len(out_pieces) and len(_READ_AT) * len(_STEPS) == NP
        count["writes"] = lead
        for p, (i, c) in enumerate(_STEPS):
            @pl.when(first)
            def _():
                x_wait(i * XN, c * _CHUNK, _CHUNK, 2 * B + i * chunks + c)

            if c == 0:
                @pl.when(t > 0)
                def _():
                    x_wait(xg + i * XN, col, half, 4 * k + 2 * i + h)

            def load_x(u, n, k0, j):
                window = pl.ds(c * _CHUNK + 256 * u + 128 * j, 128)
                cuts = sorted({k0, k0 + n} | set(range(-(-k0 // _XG) * _XG, k0 + n, _XG)))
                return jnp.concatenate(
                    [xs[i * XN + lo // _XG, pl.ds(lo % _XG, hi - lo), window]
                     for lo, hi in zip(cuts, cuts[1:])], axis=0)

            def store_out(u, v):
                window = pl.ds(c * _CHUNK + 256 * u, 256)
                cuts = sorted({i * F, i * F + F} | set(range(-(-i * F // _OG) * _OG, i * F + F, _OG)))
                for lo, hi in zip(cuts, cuts[1:]):
                    os_[lo // _OG, pl.ds(lo % _OG, hi - lo), window] = v[lo - i * F:hi - i * F]

            _tokens512(w1_ref, w2_ref, bias_ref, load_x, store_out, tick, plain_first=p == 0)
        write(lead, t + 1 - B // 2)
        return carry

    lax.fori_loop(0, B, step, 0)
    for piece in out_halves[1]:
        out_copy(B // 2 - 1, *piece).start()
    pltpu.make_async_copy(obuf, obuf, osem.at[0]).wait()


@jax.jit
def pallas_standalone__structured_sparse_n_m__ragged_kernel(
    x: jax.Array,
    w: jax.Array,
    b: jax.Array,
):
    B, S, D = x.shape
    F = w.shape[1]
    xt = jnp.transpose(x, (0, 2, 1)).reshape(B * D // _XG, _XG, S)
    out = pl.pallas_call(
        _kernel,
        in_specs=[pl.BlockSpec(memory_space=pl.ANY)] * 3,
        out_specs=pl.BlockSpec(memory_space=pl.ANY),
        out_shape=jax.ShapeDtypeStruct((B * F // _OG, _OG, S), x.dtype),
        scratch_shapes=[
            pltpu.VMEM((2 * _XRING * D // _XG, _XG, S), x.dtype),
            pltpu.VMEM((B * F // _OG, _OG, S), x.dtype),
            pltpu.VMEM((D, F), w.dtype),
            pltpu.VMEM((F,), b.dtype),
            pltpu.VMEM((len(_SINGLE), F // 4, 128), I32),
            pltpu.VMEM((7 * len(_DOUBLE), F // 8, 128), I32),
            pltpu.VMEM((F, 128), F32),
            pltpu.SemaphoreType.DMA((2 * B + S // _CHUNK,)),
            pltpu.SemaphoreType.DMA((1,)),
            pltpu.SemaphoreType.DMA((1 + len(_W_ROWS),)),
        ],
        compiler_params=pltpu.CompilerParams(
            vmem_limit_bytes=124 * 1024 * 1024,
            flags={"XLA_TPU_RESCHEDULE_DMA_DONES": True},
            disable_bounds_checks=True,
            disable_semaphore_checks=True,
        ),
    )(xt, w, b)
    return jnp.transpose(out.reshape(B, F, S), (0, 2, 1))
```

```python
import jax
import jax.numpy as jnp
from jax import lax
import jax.experimental.pallas as pl
import jax.experimental.pallas.tpu as pltpu

F32, BF16, I32 = jnp.float32, jnp.bfloat16, jnp.int32

_PASSES = {
    "Gp": [(96, {(0, 0): 1, (1, 128): 1}, {(0, 0): 1, (128, 1): 1}),
           (32, {(0, 352): 1, (1, 480): -1}, {(352, 0): 1, (480, 1): -1})],
    "Gm": [(96, {(0, 256): 1, (1, 384): 1}, {(256, 0): 1, (384, 1): -1}),
           (32, {(0, 96): 1, (1, 224): -1}, {(96, 0): 1, (224, 1): 1})],
    "R0p": [(128, {(0, 256): 1, (0, 384): 1}, {(384, 1): 1})],
    "R0m": [(128, {(0, 0): 1, (0, 128): 1}, {(128, 1): 1})],
    "R1p": [(128, {(1, 256): 1, (1, 384): 1}, {(256, 0): 1})],
    "R1m": [(128, {(1, 0): 1, (1, 128): 1}, {(0, 0): 1})],
    "C0m": [(64, {(0, 512): 0.5, (1, 512): -0.5}, {(512, 0): 1}),
            (32, {(1, 224): 1}, {(96, 0): 1, (224, 0): -1}),
            (32, {(1, 480): 1}, {(352, 0): 1, (480, 0): -1})],
    "C1m": [(64, {(0, 512): 0.5, (1, 512): -0.5}, {(512, 1): 1}),
            (32, {(0, 96): 1}, {(96, 1): 1, (224, 1): -1}),
            (32, {(0, 352): 1}, {(352, 1): 1, (480, 1): -1})],
    "C0a": [(96, {(1, 128): 1}, {(128, 0): 1, (0, 0): -1}),
            (32, {(0, 512): 0.5, (1, 512): 0.5}, {(512, 0): 1})],
    "C0b": [(96, {(1, 384): 1}, {(384, 0): 1, (256, 0): -1}),
            (32, {(0, 544): 0.5, (1, 544): 0.5}, {(544, 0): 1})],
    "C1a": [(96, {(0, 0): 1}, {(0, 1): 1, (128, 1): -1}),
            (32, {(0, 512): 0.5, (1, 512): 0.5}, {(512, 1): 1})],
    "C1b": [(96, {(0, 256): 1}, {(256, 1): 1, (384, 1): -1}),
            (32, {(0, 544): 0.5, (1, 544): 0.5}, {(544, 1): 1})],
    "D0a": [(96, {(0, 128): 1, (1, 128): -1}, {(128, 0): 1, (128, 1): 1}),
            (32, {(0, 224): 1, (1, 224): 1}, {(224, 0): 1, (224, 1): 1})],
    "D0b": [(96, {(0, 384): 1, (1, 384): -1}, {(384, 0): 1, (384, 1): -1}),
            (32, {(0, 480): 1, (1, 480): 1}, {(480, 0): 1, (480, 1): -1})],
    "D1a": [(96, {(1, 0): 1, (0, 0): -1}, {(0, 0): 1, (0, 1): 1}),
            (32, {(1, 96): 1, (0, 96): 1}, {(96, 0): 1, (96, 1): 1})],
    "D1b": [(96, {(0, 256): 1, (1, 256): -1}, {(256, 0): 1, (256, 1): -1}),
            (32, {(1, 352): -1, (0, 352): -1}, {(352, 0): 1, (352, 1): -1})],
}
_SINGLE = ("Gp", "Gm", "R0p", "R0m", "R1p", "R1m", "C0m", "C1m")
_DOUBLE = ("C0", "C1", "D0", "D1")

_XG = 64
_OG = 128
_CHUNK = 512
_OCHUNK = 1024
_XRING = 5
_W_ROWS = ((512, 64), (0, 128), (128, 128), (256, 128), (384, 128))
_ORDER = ((0, 0), (0, 1), (1, 0), (1, 1), (0, 2), (1, 2), (0, 3), (1, 3))
_TICKS = 60
_READ_AT = (0, 8, 16, 24, 28, 36, 44, 52)
_WRITE_AT = {36: 2, 52: 6}
_LATE = 5


def _cut(lo, hi, n):
    cuts = [lo, *range(lo - lo % n + n, hi, n), hi]
    return list(zip(cuts, cuts[1:]))


def _prune(w):
    words = pltpu.bitcast(w, I32)
    mate = lax.broadcasted_iota(I32, (8, w.shape[1]), 0) ^ 1
    parts = []
    for i in range(0, words.shape[0], 8):
        u = words[i:i + 8]
        lo = pltpu.bitcast((u << 16) & 0x7FFFFFFF, F32)
        hi = pltpu.bitcast(u & 0x7FFF0000, F32)
        big, small = jnp.maximum(lo, hi), jnp.minimum(lo, hi)
        nbig = jnp.take_along_axis(big, mate, axis=0, mode="promise_in_bounds")
        nsmall = jnp.take_along_axis(small, mate, axis=0, mode="promise_in_bounds")
        thr = jnp.maximum(jnp.minimum(big, nbig), jnp.maximum(small, nsmall))
        parts.append(u & (jnp.where(lo < thr, 0, 0xFFFF) | jnp.where(hi < thr, 0, -65536)))
    return pltpu.bitcast(jnp.concatenate(parts, axis=0), BF16)


def _prepare_weights(w_copies, b_copy, wbuf, bbuf, w1_ref, w2_ref, bias_ref):
    F = wbuf.shape[1]
    H = F // 2
    tiles = {}
    for cp, (k0, n) in zip(w_copies, _W_ROWS):
        cp.wait()
        wp = _prune(wbuf[k0:k0 + n, :])
        if n < 128:
            b_copy.wait()
            bias = jnp.broadcast_to(bbuf[...].reshape(1, F).astype(F32), (128 - n, F))
            wp = jnp.concatenate([wp, bias.astype(BF16)], axis=0)
        tiles[k0] = wp.T
    tiles = {k0: t.astype(F32) for k0, t in tiles.items()}
    low = lax.broadcasted_iota(I32, (F, 128), 1) < 64
    bias_ref[...] = jnp.where(low, pltpu.roll(tiles[512], 64, 1), tiles[512])
    lane = lax.broadcasted_iota(I32, (H, 128), 1)

    def operand(name):
        pos, res = 0, None
        for depth, coefs, _ in _PASSES[name]:
            ((i, k), scale), *rest = coefs.items()
            v = tiles[k - k % 128][i * H:(i + 1) * H]
            for (i2, k2), c in rest:
                t = tiles[k2 - k2 % 128][i2 * H:(i2 + 1) * H]
                v = v + t if c == scale else v - t
            if scale != 1:
                v = v * scale
            if k % 128 != pos:
                v = pltpu.roll(v, (pos - k) % 128, 1)
            res = v if res is None else jnp.where(lane < pos, res, v)
            pos += depth
        return res

    for p, name in enumerate(_SINGLE):
        w1_ref[p] = pltpu.bitcast(operand(name).astype(BF16), I32)
    for p, name in enumerate(_DOUBLE):
        a, b = operand(name + "a"), operand(name + "b")
        a0, a1, b0, b1 = a[:H // 2], a[H // 2:], b[:H // 2], b[H // 2:]
        for i, v in enumerate((a1 + b1, b1, a0 + b1, b0 - b1, a0 + b0, a0, a0 - a1)):
            w2_ref[7 * p + i] = pltpu.bitcast(v.astype(BF16), I32)


def _tokens512(w1_ref, w2_ref, bias_ref, load_x, store_out, tick, plain_first):
    H = bias_ref.shape[0] // 2

    def x_operand(name, u):
        parts = []
        for depth, _, signs in _PASSES[name]:
            (first, _), *rest = signs.items()
            v = load_x(u, depth, *first)
            for other, sign in rest:
                v, q = v.astype(F32), load_x(u, depth, *other).astype(F32)
                v = v + q if sign > 0 else v - q
            parts.append(v)
        return parts

    def dot(w, parts):
        x = jnp.concatenate([p.astype(BF16) for p in parts], axis=0)
        return jnp.dot(pltpu.bitcast(w, BF16), x, preferred_element_type=F32)

    def single(name, u):
        tick(2)
        return dot(w1_ref[_SINGLE.index(name)], x_operand(name, u))

    def double(name):
        u, v = (0, 1) if name[0] == "C" else (1, 0)
        xa, xb = name + "a", name + "b"

        def m(i, p, q=None):
            tick(1)
            parts = x_operand(*p)
            if q is not None:
                parts = [s.astype(F32) - t.astype(F32) for s, t in zip(parts, x_operand(*q))]
            return dot(w2_ref[7 * _DOUBLE.index(name) + i], parts)

        m2, m4 = m(0, (xa, u)), m(1, (xb, u), (xa, u))
        m1, m7 = m(2, (xa, u), (xb, v)), m(3, (xb, u), (xb, v))
        low_u, top_u, low_v = m2 + m4, (m1 + m4) + m7, m2 - m1
        m5, m3, m6 = m(4, (xb, v)), m(5, (xa, v), (xb, v)), m(6, (xa, u), (xa, v))
        return {u: jnp.concatenate([top_u + m5, low_u], axis=0),
                v: jnp.concatenate([m3 + m5, (m3 + m6) + low_v], axis=0)}

    def rows(u):
        p0, m0 = single("R0p", u) + bias_ref[0:H, :], single("R0m", u)
        p1, m1 = single("R1p", u) + bias_ref[H:, :], single("R1m", u)
        return p0 - m0, p0 + m0, p1 + m1, p1 - m1

    def rest(u, c0, c1, d0, d1):
        gp, gm, m0, m1 = (single(name, u) for name in ("Gp", "Gm", "C0m", "C1m"))
        return (((gp + gm) + m0) + (c0[u] + d0[u]), c1[u] + m1,
                c0[u] - m0, ((gp - gm) - m1) + (c1[u] + d1[u]))

    done = {0: rows(0)} if plain_first else {}
    doubles = [double(name) for name in _DOUBLE]
    for u in range(2):
        c = rest(u, *doubles)
        c = [s + t for s, t in zip(c, done[u] if u in done else rows(u))]
        halves = [jnp.concatenate(c[i:i + 2], axis=1).astype(BF16) for i in (0, 2)]
        store_out(u, jnp.concatenate(halves, axis=0))


def _kernel(x_hbm, w_hbm, b_hbm, o_hbm, xbuf, obuf, wbuf, bbuf, w1_ref, w2_ref, bias_ref,
            xsem, osem, wsem):
    D, F = w_hbm.shape
    S = x_hbm.shape[2]
    XN, ON = D // _XG, 2 * F // _OG
    B = x_hbm.shape[0] // XN
    half = S // 2
    tiles = _XG // 8
    chunks = half // _CHUNK
    pieces = [(8 * r, _CHUNK * c) for r in range(tiles) for c in range(2 * chunks)]
    early = ([(8 * r, _CHUNK * c) for c in range(chunks) for r in range(tiles)]
             + [p for p in pieces if p[1] >= half])
    NP = len(pieces)

    def select(pred, p, q, col_align):
        row, col = (jnp.where(pred, a, b) for a, b in zip(p, q))
        return pl.multiple_of(row, 8), pl.multiple_of(col, col_align)

    def ring(k):
        return jnp.where(k >= _XRING, k - _XRING, k)

    def x_copy(k, i, row, col, sem):
        window = (pl.ds(row, 8), pl.ds(col, _CHUNK))
        return pltpu.make_async_copy(x_hbm.at[(pl.ds((2 * k + i) * XN, XN), *window)],
                                     xbuf.at[(pl.ds((2 * ring(k) + i) * XN, XN), *window)],
                                     xsem.at[sem])

    def x_wait(g0, col, n, sem):
        dst = xbuf.at[pl.ds(g0, XN), :, pl.ds(col, n)]
        pltpu.make_async_copy(dst, dst, xsem.at[sem]).wait()

    def out_copy(k, row, col):
        window = (pl.ds(k * ON, ON), pl.ds(row, 8), pl.ds(col, _OCHUNK))
        return pltpu.make_async_copy(obuf.at[window], o_hbm.at[window], osem.at[0])

    out_pieces = [(r, c) for r in range(0, _OG, 8) for c in range(0, S, _OCHUNK)]
    out_halves = [[p for p in out_pieces if p[1] // half == h] for h in range(2)]

    b_copy = pltpu.make_async_copy(b_hbm, bbuf, wsem.at[0])
    w_copies = [pltpu.make_async_copy(w_hbm.at[pl.ds(k0, n)], wbuf.at[pl.ds(k0, n)], wsem.at[1 + i])
                for i, (k0, n) in enumerate(_W_ROWS)]
    b_copy.start()
    for cp in w_copies:
        cp.start()

    def first_reads(c, carry):
        for r in range(tiles):
            x_copy(0, 0, 8 * r, pl.multiple_of(c * _CHUNK, _CHUNK), 2 * B + c).start(priority=1)
        return carry

    lax.fori_loop(0, chunks, first_reads, 0)
    _prepare_weights(w_copies, b_copy, wbuf, bbuf, w1_ref, w2_ref, bias_ref)

    def step(t, carry):
        k, h = t >> 1, t & 1
        first = t == 0
        xg = 2 * XN * ring(k)
        col = pl.multiple_of(h * half, half)
        x_view = xbuf.at[pl.ds(xg, 2 * XN), :, pl.ds(col, half)]
        o_view = obuf.at[pl.ds(k * ON, ON), :, pl.ds(col, half)]
        count = {"ticks": 0, "reads": 0, "writes": 0}

        def read():
            i = count["reads"]
            count["reads"] += 1
            ahead, j = divmod(i + NP // 2, NP)

            @pl.when(t < B // 2 - int(i >= NP - _LATE))
            def _():
                sem = 2 * B + chunks + i // tiles if early[i][1] < half else 3
                sem = jnp.where(first, sem, 4 * t + 2 + pieces[i][1] // half)
                x_copy(t, 1, *select(first, early[i], pieces[i], _CHUNK), sem).start(priority=0)

            @pl.when(t < B // 2 - ahead)
            def _():
                sem = 4 * (t + ahead) + pieces[j][1] // half
                if ahead:
                    x_copy(t + 1, 0, *pieces[j], sem).start(priority=1)
                else:
                    x_copy(t, 0, *select(first, early[j], pieces[j], _CHUNK),
                           jnp.where(first, 1, sem)).start(priority=1)

            if ahead and j < _LATE:
                @pl.when(t == B // 2 - 1)
                def _():
                    row, c = pieces[NP - _LATE + j]
                    x_copy(t, 1, row, c, 4 * t + 2 + c // half).start(priority=1)

        def write(n, pair):
            for _ in range(n):
                i = count["writes"] % len(out_pieces)
                count["writes"] += 1
                last = i < len(out_halves[0])

                @pl.when((pair >= 0) & (pair < B // 2 - 1 + last))
                def _():
                    piece = out_pieces[i]
                    if last:
                        piece = select(pair == B // 2 - 1, out_halves[0][i], piece, _OCHUNK)
                    out_copy(pair, *piece).start()

        def tick(n):
            pos = count["ticks"] % _TICKS
            count["ticks"] += n
            write(_WRITE_AT.get(pos, 0) * (count["writes"] < len(out_pieces)), t - B // 2)
            if pos in _READ_AT:
                read()

        lead = sum(_WRITE_AT.values())
        assert lead * len(_ORDER) == len(out_pieces) and len(_READ_AT) * len(_ORDER) == NP
        count["writes"] = lead
        for p, (i, c) in enumerate(_ORDER):
            @pl.when(first)
            def _():
                x_wait(i * XN, c * _CHUNK, _CHUNK, 2 * B + i * chunks + c)

            if c == 0:
                @pl.when(t > 0)
                def _():
                    x_wait(xg + i * XN, col, half, 4 * k + 2 * i + h)

            def load_x(u, n, k0, j):
                window = pl.ds(c * _CHUNK + 256 * u + 128 * j, 128)
                return jnp.concatenate(
                    [x_view[i * XN + lo // _XG, pl.ds(lo % _XG, hi - lo), window]
                     for lo, hi in _cut(k0, k0 + n, _XG)], axis=0)

            def store_out(u, v):
                window = pl.ds(c * _CHUNK + 256 * u, 256)
                for lo, hi in _cut(i * F, (i + 1) * F, _OG):
                    o_view[lo // _OG, pl.ds(lo % _OG, hi - lo), window] = v[lo - i * F:hi - i * F]

            _tokens512(w1_ref, w2_ref, bias_ref, load_x, store_out, tick, plain_first=p == 0)
        write(lead, t + 1 - B // 2)
        return carry

    lax.fori_loop(0, B, step, 0)
    for piece in out_halves[1]:
        out_copy(B // 2 - 1, *piece).start()
    pltpu.make_async_copy(obuf, obuf, osem.at[0]).wait()


@jax.jit
def pallas_standalone__structured_sparse_n_m__ragged_kernel(
    x: jax.Array,
    w: jax.Array,
    b: jax.Array,
):
    B, S, D = x.shape
    F = w.shape[1]
    xt = jnp.transpose(x, (0, 2, 1)).reshape(B * D // _XG, _XG, S)
    out = pl.pallas_call(
        _kernel,
        in_specs=[pl.BlockSpec(memory_space=pl.ANY)] * 3,
        out_specs=pl.BlockSpec(memory_space=pl.ANY),
        out_shape=jax.ShapeDtypeStruct((B * F // _OG, _OG, S), x.dtype),
        scratch_shapes=[
            pltpu.VMEM((2 * _XRING * D // _XG, _XG, S), x.dtype),
            pltpu.VMEM((B * F // _OG, _OG, S), x.dtype),
            pltpu.VMEM((D, F), w.dtype),
            pltpu.VMEM((F,), b.dtype),
            pltpu.VMEM((len(_SINGLE), F // 4, 128), I32),
            pltpu.VMEM((7 * len(_DOUBLE), F // 8, 128), I32),
            pltpu.VMEM((F, 128), F32),
            pltpu.SemaphoreType.DMA((2 * B + S // _CHUNK,)),
            pltpu.SemaphoreType.DMA((1,)),
            pltpu.SemaphoreType.DMA((1 + len(_W_ROWS),)),
        ],
        compiler_params=pltpu.CompilerParams(
            vmem_limit_bytes=124 * 1024 * 1024,
            flags={"XLA_TPU_RESCHEDULE_DMA_DONES": True},
            disable_bounds_checks=True,
            disable_semaphore_checks=True,
        ),
    )(xt, w, b)
    return jnp.transpose(out.reshape(B, F, S), (0, 2, 1))
```
